```python
import os as _os
_os.environ.setdefault('JAX_PLATFORMS', 'cpu')
import jax
import jax.numpy as jnp

def _softmax(x, axis=-1):
    return jax.nn.softmax(x, axis=axis)

def _gelu(x):
    return jax.nn.gelu(x, approximate=True)

def _silu(x):
    return jax.nn.silu(x)

def _sigmoid(x):
    return jax.nn.sigmoid(x)

def _layernorm(x, axis=-1, eps=1e-05):
    m = jnp.mean(x, axis=axis, keepdims=True)
    v = jnp.var(x, axis=axis, keepdims=True)
    return (x - m) / jnp.sqrt(v + eps)

def _scatter_add(tgt, idx, src, axis=0):
    return tgt.at[idx].add(src)

def _segment_sum(src, seg, n):
    return jax.ops.segment_sum(src, seg, n)

class _Rng:

    def __init__(self, key):
        self._k = key

    def _next(self):
        self._k, sub = jax.random.split(self._k)
        return sub

    def normal(self, shape):
        return jax.random.normal(self._next(), shape, dtype=jnp.bfloat16)

    def randint(self, lo, hi, shape):
        return jax.random.randint(self._next(), shape, lo, hi, dtype=jnp.int32)

    def uniform(self, shape, lo=0.0, hi=1.0):
        return jax.random.uniform(self._next(), shape, jnp.bfloat16, lo, hi)

    def permutation(self, n):
        return jax.random.permutation(self._next(), n)
kernel_name = 'concat_heads__spectral_gfnet__memory_aug_recurrent_mem_tr__prompt'

def setup_inputs():
    _rng = _Rng(jax.random.key(int.from_bytes(__import__("os").urandom(4), "little")))
    _w = lambda a: (lambda t: t.astype(jnp.bfloat16) if jnp.issubdtype(t.dtype, jnp.floating) else t)(jnp.asarray(a))

    def _A_setup():
        B, S, D = (1, 2048, 512)
        Df = D // 2 + 1
        return {'x': _w((lambda *s: _rng.normal(s) * 0.05)(B, S, D)), 'w_r': _w((lambda *s: _rng.normal(s) * 0.05)(S, Df) * 0.02), 'w_i': _w((lambda *s: _rng.normal(s) * 0.05)(S, Df) * 0.02)}
    _A_in = _A_setup()

    def _B_setup():
        B, S, Dm = (1, 2048, 512)
        H, Dh = (32, 128)
        M, seg = (8, 32)
        seg = min(seg, S)
        S = S // seg * seg
        return {'x': _w((lambda *s: _rng.normal(s) * 0.05)(B, S, Dm)), 'mem0': _w((lambda *s: _rng.normal(s) * 0.4)(B, M, Dm)), 'Wq': _w((lambda *s: _rng.normal(s) * 3.2)(Dm, H, Dh) * Dm ** (-0.5)), 'Wk': _w((lambda *s: _rng.normal(s) * 3.2)(Dm, H, Dh) * Dm ** (-0.5)), 'Wv': _w((lambda *s: _rng.normal(s) * 0.4)(Dm, H, Dh) * Dm ** (-0.5)), 'Wo': _w((lambda *s: _rng.normal(s) * 0.4)(H, Dh, Dm) * (H * Dh) ** (-0.5)), 'seg_len': seg}
    _B_in = _B_setup()
    return {'A_x': _A_in['x'], 'A_w_r': _A_in['w_r'], 'A_w_i': _A_in['w_i'], 'B_x': _B_in['x'], 'B_mem0': _B_in['mem0'], 'B_Wq': _B_in['Wq'], 'B_Wk': _B_in['Wk'], 'B_Wv': _B_in['Wv'], 'B_Wo': _B_in['Wo'], 'B_seg_len': _B_in['seg_len']}

def reference(A_x, A_w_r, A_w_i, B_x, B_mem0, B_Wq, B_Wk, B_Wv, B_Wo, B_seg_len):

    def _A_ref(x, w_r, w_i):
        B, S, D = x.shape
        X = (lambda x, axes=(-2, -1): jnp.fft.rfft2(x.astype(jnp.float32), axes=axes))(x, axes=(-2, -1))
        W = w_r + 1j * w_i
        X = X * W
        y = (lambda x, s, axes=(-2, -1): jnp.fft.irfft2(x, s=s, axes=axes).astype(jnp.bfloat16))(X, (S, D), axes=(-2, -1))
        return y

    def _B_ref(x, mem0, Wq, Wk, Wv, Wo, seg_len):
        B, S, Dm = x.shape
        H, Dh = (Wq.shape[1], Wq.shape[2])
        M = mem0.shape[1]
        scale = Dh ** (-0.5)
        n_seg = S // seg_len
        L = M + seg_len
        idx = jnp.arange(L)
        mask = (idx[:, None] < M) | (idx[:, None] >= idx[None, :])
        mem = mem0
        outs = []
        for s in range(n_seg):
            xs = x[:, s * seg_len:(s + 1) * seg_len, :].copy()
            h = jnp.concatenate([mem, xs], axis=1)
            q = jnp.einsum('btd,dhe->bhte', h, Wq)
            k = jnp.einsum('btd,dhe->bhte', h, Wk)
            v = jnp.einsum('btd,dhe->bhte', h, Wv)
            scores = jnp.einsum('bhqe,bhke->bhqk', q, k) * scale
            scores = jnp.where(mask[None, None], scores, -1000000000.0)
            p = _softmax(scores, axis=-1)
            o = jnp.einsum('bhqk,bhke->bhqe', p, v)
            o = jnp.einsum('bhte,hed->btd', o, Wo)
            mem = o[:, :M, :].copy()
            outs.append(o[:, M:, :])
        return jnp.concatenate(outs, axis=1)
    a = _A_ref(A_x, A_w_r, A_w_i)
    b = _B_ref(B_x, B_mem0, B_Wq, B_Wk, B_Wv, B_Wo, B_seg_len)
    return jnp.concatenate([a, b], axis=-1)
```

```python
import itertools

import jax
import jax.numpy as jnp
import numpy as np
from jax import lax
from jax.experimental import pallas as pl
from jax.experimental.pallas import tpu as pltpu

F32, BF16, U32 = jnp.float32, jnp.bfloat16, jnp.uint32
SEQ, DM, HEADS, DH, NMEM, SEG = 2048, 512, 32, 128, 8, 32
NSEG = SEQ // SEG
LEN = NMEM + SEG
LOG2E = 1.4426950408889634

STRASSEN = (
    ({(0, 0): 1, (1, 1): 1}, {(0, 0): 1, (1, 1): 1}, {(0, 0): 1, (1, 1): 1}),
    ({(1, 0): 1, (1, 1): 1}, {(0, 0): 1}, {(1, 0): 1, (1, 1): -1}),
    ({(0, 0): 1}, {(0, 1): 1, (1, 1): -1}, {(0, 1): 1, (1, 1): 1}),
    ({(1, 1): 1}, {(1, 0): 1, (0, 0): -1}, {(0, 0): 1, (1, 0): 1}),
    ({(0, 0): 1, (0, 1): 1}, {(1, 1): 1}, {(0, 0): -1, (0, 1): 1}),
    ({(1, 0): 1, (0, 0): -1}, {(0, 0): 1, (0, 1): 1}, {(1, 1): 1}),
    ({(0, 1): 1, (1, 1): -1}, {(1, 0): 1, (1, 1): 1}, {(0, 0): 1}),
)
PHASE = ((4, 2, 6, 0), (1, 3, 5, 0))
NPROD = 49
PRODS = tuple(itertools.product(range(7), range(7)))


def _rows_in_step(a, b, s):
    st = [2 * p + q for p in range(2) for q in range(2) if a in PHASE[p] and b in PHASE[q]]
    k = st.index(s)
    return k * 4 // len(st), (k + 1) * 4 // len(st)


def _touch():
    t = {}
    for s in range(4):
        for a in PHASE[s >> 1]:
            for b in PHASE[s & 1]:
                for (r1, n1) in STRASSEN[a][2]:
                    for (r2, n2) in STRASSEN[b][2]:
                        l = t.setdefault((2 * r1 + r2, 2 * n1 + n2), [])
                        if s not in l:
                            l.append(s)
    return t


TOUCH = _touch()


def _lin(terms):
    terms = sorted(terms, key=lambda t: -t[0])
    c, x = terms[0]
    acc = x if c > 0 else -x
    for c, x in terms[1:]:
        acc = acc + x if c > 0 else acc - x
    return acc


def _lin_rows(terms):
    cuts = sorted({v for _, (lo, hi, _x) in terms for v in (lo, hi)})
    parts = []
    for lo, hi in zip(cuts[:-1], cuts[1:]):
        sel = []
        for c, (l, h, x) in terms:
            if l <= lo and hi <= h:
                sel.append((c, x if (l, h) == (lo, hi) else x[8 * (lo - l):8 * (hi - l)]))
        parts.append(_lin(sel))
    return cuts[0], cuts[-1], parts[0] if len(parts) == 1 else jnp.concatenate(parts, 0)


def _token_blocks(tok, outer, inner):
    mid = {}
    for a in outer:
        for rn in itertools.product(range(2), range(2)):
            tm = [(STRASSEN[b][2][rn], tok[a, b]) for b in inner
                  if rn in STRASSEN[b][2] and (a, b) in tok]
            if tm:
                mid[a, rn] = _lin_rows(tm)
    for r1, n1, r2, n2 in itertools.product(range(2), repeat=4):
        tm = [(STRASSEN[a][2][r1, n1], mid[a, (r2, n2)]) for a in outer
              if (r1, n1) in STRASSEN[a][2] and (a, (r2, n2)) in mid]
        if tm:
            yield (2 * r1 + r2, 2 * n1 + n2), tm


def _mem_blocks(mem, s):
    p, q = s >> 1, s & 1
    mid = {(a, n): _lin([(STRASSEN[b][2][q, n], mem[a, b]) for b in PHASE[q] if (q, n) in STRASSEN[b][2]])
           for a in PHASE[p] for n in range(2)}
    return [_lin([(STRASSEN[a][2][p, n1], mid[a, n2]) for a in PHASE[p] if (p, n1) in STRASSEN[a][2]])
            for n1 in range(2) for n2 in range(2)]


def _mem_lhs(a, b, s, m):
    return _lin([(ca * cb, m[2 * c1 + c2])
                 for (r1, c1), ca in STRASSEN[a][0].items() if r1 == s >> 1
                 for (r2, c2), cb in STRASSEN[b][0].items() if r2 == s & 1])


def _mm(a, b):
    return jnp.dot(a, b, preferred_element_type=F32)


def _mm_nt(a, b):
    return lax.dot_general(a, b, (((1,), (1,)), ((), ())), preferred_element_type=F32)


def _lo(u):
    return lax.bitcast_convert_type(u << 16, F32)


def _hi(u):
    return lax.bitcast_convert_type(u & np.uint32(0xFFFF0000), F32)


def _pack(x):
    return pltpu.bitcast(x.astype(BF16), U32)


def _twiddle(z, k, sign):
    k = (k * sign) % 16
    re, im = z
    if k == 0:
        return re, im
    if k == 4:
        return -im, re
    if k == 8:
        return -re, -im
    if k == 12:
        return im, -re
    c, s = float(np.cos(np.pi * k / 8)), float(np.sin(np.pi * k / 8))
    if k % 4 == 2:
        if c * s > 0:
            return (re - im) * c, (re + im) * c
        return (re + im) * c, (im - re) * c
    return re * c - im * s, re * s + im * c


def _dft4(z, sign):
    (ar, ai), (br, bi), (cr, ci), (dr, di) = z
    pr, pi, mr, mi = ar + cr, ai + ci, ar - cr, ai - ci
    qr, qi, nr, ni = br + dr, bi + di, br - dr, bi - di
    up, dn = (mr - ni, mi + nr), (mr + ni, mi - nr)
    return [(pr + qr, pi + qi), up if sign > 0 else dn, (pr - qr, pi - qi), dn if sign > 0 else up]


def _dft16(z, sign):
    cols = [_dft4([z[n2 + 4 * n1] for n1 in range(4)], sign) for n2 in range(4)]
    out = [None] * 16
    for k1 in range(4):
        r = _dft4([_twiddle(cols[n2][k1], n2 * k1, sign) for n2 in range(4)], sign)
        for k2 in range(4):
            out[k1 + 4 * k2] = r[k2]
    return out


def _dft_constants():
    n = np.arange(128)[None, :]
    k = np.arange(64)[:, None]

    def cs(r):
        th = 2 * np.pi * ((n * (4 * k + r)) % 512) / 512
        return np.cos(th), np.sin(th)

    c0, s0 = cs(0)
    c1, s1 = cs(1)
    c2, s2 = cs(2)
    c3, s3 = cs(3)
    f0 = np.concatenate([c0, -s0])
    f0[64] = np.cos(np.pi * n[0])
    fwd = np.stack([f0, np.concatenate([c2, -s2]),
                    np.concatenate([c1, -s1]), np.concatenate([c3, -s3]),
                    np.concatenate([-s1, -c1]), np.concatenate([s3, c3])])
    inv = fwd * (2.0 / (SEQ * DM))
    inv[0, 0] *= 0.5
    inv[0, 64] *= 0.5
    a = np.arange(16)[:, None, None]
    b = np.arange(128)[None, :, None]
    ph = 2 * np.pi * (((a + 16 * b) * n[None]) % SEQ) / SEQ
    g = np.stack([np.cos(ph), -np.sin(ph)], 1).reshape(32, 128, 128)
    consts = np.concatenate([fwd, inv, g]).astype(np.float32)
    u = consts.view(np.uint32)
    h = (u + 0x7FFF + ((u >> 16) & 1)) >> 16
    return (h[:, 0::2] | (h[:, 1::2] << 16)).astype(np.uint32)


DFT_CONSTS = _dft_constants()
C_FWD, C_INV, C_G = 0, 6, 12
ZROWS = 264


def _spectral_forward(xa, cst, z_re, z_im):
    xu = xa
    first = lax.broadcasted_iota(jnp.int32, (8, 128), 0) == 0
    const = lambda i: pltpu.bitcast(cst[i], BF16)

    @pl.loop(0, 8)
    def _(j):
        words = [xu[c, pl.ds(j, 128, stride=8), :] for c in range(4)]
        for half, unpack in enumerate((_lo, _hi)):
            a = 2 * j + half
            x0, x1, x2, x3 = [unpack(w) for w in words]
            p, q = x0 + x2, x1 + x3
            r0 = _mm_nt(const(C_FWD), (p + q).astype(BF16))
            r2 = _mm_nt(const(C_FWD + 1), (p - q).astype(BF16))
            u, w = (x0 - x2).astype(BF16), (x1 - x3).astype(BF16)
            odd = (_mm_nt(jnp.concatenate([const(C_FWD + 2), const(C_FWD + 3)], 0), u)
                   + _mm_nt(jnp.concatenate([const(C_FWD + 4), const(C_FWD + 5)], 0), w))
            nyq = jnp.where(first, r0[64:72], 0.0)
            ure = jnp.concatenate([r0[:64], odd[:64], r2[:64], odd[128:192], nyq], 0)
            uim = jnp.concatenate([jnp.where(first, 0.0, r0[64:72]), r0[72:], odd[64:128], r2[64:], odd[192:]], 0)
            gr, gi = const(C_G + 2 * a), const(C_G + 2 * a + 1)
            rr, ri, ir, ii = _mm(ure, gr), _mm(ure, gi), _mm(uim, gr), _mm(uim, gi)
            z_re[a, 0:256] = rr[:256] - ii
            z_im[a, 0:256] = ri[:256] + ir
            z_re[a, 256:ZROWS] = rr[256:]
            z_im[a, 256:ZROWS] = ri[256:]


def _spectral_filter(wr, wi, wnyq, z_re, z_im):
    wru, wiu = wr, wi

    def mix(row, weight):
        z = [(z_re[a, pl.ds(row, 8), :], z_im[a, pl.ds(row, 8), :]) for a in range(16)]
        y = []
        for k, (xr, xi) in enumerate(_dft16(z, -1)):
            cr, ci = weight(k)
            y.append((xr * cr - xi * ci, xr * ci + xi * cr))
        for a, (yr, yi) in enumerate(_dft16(y, 1)):
            z_re[a, pl.ds(row, 8), :] = yr
            z_im[a, pl.ds(row, 8), :] = yi

    @pl.loop(0, 16)
    def _(i):
        odd, blk = i >> 3, i & 7
        for half, unpack in enumerate((_lo, _hi)):
            row = pl.multiple_of((2 * odd + half) * 64 + blk * 8, 8)
            src = pl.ds(16 * blk + odd, 8, stride=2)
            mix(row, lambda k: (unpack(wru[k, src, :]), unpack(wiu[k, src, :])))

    first = lax.broadcasted_iota(jnp.int32, (8, 128), 0) == 0
    mix(256, lambda k: tuple(
        jnp.where(first, wnyq[c, :, 128 * k:128 * (k + 1)].astype(F32), 0.0) for c in range(2)))


def _spectral_inverse(z_re, z_im, cst, ya):
    yu = ya
    first = lax.broadcasted_iota(jnp.int32, (8, 128), 0) == 0
    const = lambda i: pltpu.bitcast(cst[i], BF16)

    @pl.loop(0, 8)
    def _(j):
        halves = []
        for half in range(2):
            a = 2 * j + half
            gr, gi = const(C_G + 2 * a), const(C_G + 2 * a + 1)
            u = []
            for r in range(4):
                zr, zi = z_re[a, 64 * r:64 * r + 64], z_im[a, 64 * r:64 * r + 64]
                bot_r, bot_i = zi, -zr
                if r == 0:
                    bot_r = jnp.concatenate([jnp.where(first, z_re[a, 256:ZROWS], zi[:8]), zi[8:]], 0)
                    bot_i = jnp.concatenate([jnp.where(first, z_im[a, 256:ZROWS], bot_i[:8]), bot_i[8:]], 0)
                u.append(_mm_nt(gr, jnp.concatenate([zr, bot_r], 0).astype(BF16))
                         + _mm_nt(gi, jnp.concatenate([zi, bot_i], 0).astype(BF16)))
            ea, eb = _mm(u[0], const(C_INV)), _mm(u[2], const(C_INV + 1))
            oc = _mm(u[1], const(C_INV + 2)) + _mm(u[3], const(C_INV + 3))
            oe = _mm(u[1], const(C_INV + 4)) + _mm(u[3], const(C_INV + 5))
            p, q = ea + eb, ea - eb
            halves.append([lax.bitcast_convert_type(v.astype(BF16).astype(F32), U32)
                           for v in (p + oc, q + oe, p - oc, q - oe)])
        for c in range(4):
            yu[c, pl.ds(j, 128, stride=8), :] = (halves[0][c] >> 16) | halves[1][c]


def _combine_weights(load, wc, base):
    for i in range(8):
        blk = load(i)
        for a in range(7):
            mid = {(c2, n2): _lin([(v, blk[2 * c1 + c2, 2 * n1 + n2]) for (c1, n1), v in STRASSEN[a][1].items()])
                   for c2 in range(2) for n2 in range(2)}
            for b in range(7):
                wc[base + 7 * a + b, 8 * i:8 * i + 8, :] = _pack(
                    _lin([(v, mid[cn]) for cn, v in STRASSEN[b][1].items()]))


def _kernel(ax_hbm, wr_hbm, wi_hbm, x_hbm, mem_hbm, wq_hbm, wk_hbm, wv_hbm, wo_hbm, cst_hbm, out_hbm,
            xa, cst, wr, wi, wnyq, z_re, z_im, ya,
            xb, mem0, wsrc, wosrc, wc, lhs, lhs0, part, fin, o_new, o_old, yacc, yb, sems):
    lanes = lambda c: slice(128 * c, 128 * (c + 1))
    copy = pltpu.make_async_copy
    cp_ax = [copy(ax_hbm.at[:, lanes(c)], xa.bitcast(BF16).at[c], sems.at[0]) for c in range(4)]
    cp_cst = [copy(cst_hbm, cst, sems.at[1])]
    cp_w = [copy(src.at[0:256, lanes(k)], dst.bitcast(BF16).at[k], sems.at[2])
            for src, dst in ((wr_hbm, wr), (wi_hbm, wi)) for k in range(16)]
    cp_w += [copy(src.at[256:257, :], wnyq.at[c], sems.at[2]) for c, src in enumerate((wr_hbm, wi_hbm))]
    cp_x0 = [copy(x_hbm.at[0:256], xb.at[0:256], sems.at[3]), copy(mem_hbm, mem0, sems.at[3])]
    cp_qkv = [copy(src, wsrc.bitcast(BF16).at[w], sems.at[4 + w]) for w, src in enumerate((wq_hbm, wk_hbm, wv_hbm))]
    cp_wo = [copy(wo_hbm.at[:, lanes(c)], wosrc.bitcast(BF16).at[c], sems.at[7]) for c in range(4)]
    cp_x1 = [copy(x_hbm.at[256:SEQ], xb.at[256:SEQ], sems.at[8])]
    cp_ya = [copy(ya.bitcast(BF16).at[c], out_hbm.at[:, lanes(c)], sems.at[9]) for c in range(4)]

    def cp_yb(p):
        rows = pl.ds(pl.multiple_of(p * 128, 128), 128)
        return copy(yb.at[rows], out_hbm.at[rows, DM:2 * DM], sems.at[10])

    for c in cp_ax + cp_cst + cp_w + cp_x0 + cp_qkv + cp_wo + cp_x1:
        c.start()

    for c in cp_ax + cp_cst:
        c.wait()
    _spectral_forward(xa, cst, z_re, z_im)
    for c in cp_w:
        c.wait()
    _spectral_filter(wr, wi, wnyq, z_re, z_im)
    _spectral_inverse(z_re, z_im, cst, ya)
    for c in cp_ya:
        c.start()

    weight = lambda i: pltpu.bitcast(wc[i], BF16)

    def x_blocks(seg_of):
        cache = {}

        def get(r, c):
            if r not in cache:
                cache[r] = xb[pl.ds(pl.multiple_of(seg_of(r) * SEG, SEG), SEG), :].astype(F32)
            return cache[r][:, lanes(c)]
        return get

    def a_side(get):
        cache = {}

        def combo(a, b):
            tm = []
            for (r2, c2), cb in STRASSEN[b][0].items():
                if (a, r2, c2) not in cache:
                    cache[a, r2, c2] = _lin([(ca, get(2 * r1 + r2, 2 * c1 + c2))
                                             for (r1, c1), ca in STRASSEN[a][0].items()])
                tm.append((cb, cache[a, r2, c2]))
            return _lin(tm)
        return combo

    for c in cp_x0:
        c.wait()
    o_new[...] = jnp.zeros(o_new.shape, F32)
    combo0 = a_side(x_blocks(lambda r: max(r - 1, 0)))
    first_prods = [(a, b) for a, b in PRODS
                   if any(r1 or r2 for (r1, _n1) in STRASSEN[a][2] for (r2, _n2) in STRASSEN[b][2])]
    for a, b in first_prods:
        lhs0[7 * a + b] = combo0(a, b)
    wsu = wsrc

    @pl.loop(0, 24)
    def _(g):
        for w in range(3):
            @pl.when(g == 8 * w)
            def _():
                cp_qkv[w].wait()
        w, t = g >> 3, g & 7

        def load(i):
            blk = {}
            for kt in range(4):
                for n1 in range(2):
                    u = wsu[w, pl.ds((128 * kt + 16 * i) * 16 + 2 * t + n1, 16, stride=16), :]
                    blk[kt, 2 * n1], blk[kt, 2 * n1 + 1] = _lo(u), _hi(u)
            return blk
        _combine_weights(load, wc, g * NPROD)
        tok = {(a, b): (0, 4, _mm(lhs0[7 * a + b], weight(g * NPROD + 7 * a + b))) for a, b in first_prods}
        for (r, n), tm in _token_blocks(tok, range(7), range(7)):
            if r:
                fin[g, 4 * r + n] = _lin_rows(tm)[2]

    for c in cp_wo:
        c.wait()
    wou = wosrc

    @pl.loop(0, 8)
    def _(t):
        def load(i):
            return {(hd, n): pltpu.bitcast(
                wou[n, pl.ds(pl.multiple_of((4 * t + hd) * 64 + 8 * i, 8), 8), :], BF16).astype(F32)
                for hd in range(4) for n in range(4)}
        _combine_weights(load, wc, (24 + t) * NPROD)

    for c in cp_x1:
        c.wait()

    row = lax.broadcasted_iota(jnp.int32, (LEN, 48), 0)
    col = lax.broadcasted_iota(jnp.int32, (LEN, 48), 1)
    keep = ((row >= SEG) | (col >= SEG) | (row >= col)) & (col < LEN)
    fill = jnp.where(col < LEN, -1e9 * LOG2E, -jnp.inf).astype(F32)
    scale = DH ** -0.5 * LOG2E
    pad = jnp.zeros((8, 128), F32)

    def out_rows(p, r):
        return pl.ds(pl.multiple_of(p * 128 + r * SEG, SEG), SEG)

    def step(p, s, mem):
        outer, inner = PHASE[s >> 1], PHASE[s & 1]
        prods = [(a, b) for a in outer for b in inner]
        span = {ab: _rows_in_step(*ab, s) for ab in prods}
        combo = a_side(x_blocks(lambda r: jnp.minimum(4 * p + 3 + r, NSEG - 1)))
        for i, ab in enumerate(prods):
            lo, hi = span[ab]
            lhs[i, 0:8 * (hi - lo)] = combo(*ab)[8 * lo:8 * hi]
            lhs[i, 8 * (hi - lo):8 * (hi - lo) + 8] = _mem_lhs(*ab, s, mem)
        slot = (s + 1) % 4
        qkv_mem, probs, o_mem, acc = {}, {}, {}, {}

        def split(res):
            tok = {ab: (*span[ab], r[:-8]) for ab, r in res.items()}
            return tok, {ab: r[-8:] for ab, r in res.items()}

        def project(t, w):
            g = 8 * w + t
            tok, mres = split({ab: _mm(lhs[i, 0:8 * (span[ab][1] - span[ab][0]) + 8],
                                       weight(g * NPROD + 7 * ab[0] + ab[1]))
                               for i, ab in enumerate(prods)})
            for (r, n), tm in _token_blocks(tok, outer, inner):
                st = TOUCH[r, n]
                if s != st[0]:
                    tm = [(1, (0, 4, part[g, 4 * r + n]))] + tm
                (fin if s == st[-1] else part)[g, 4 * r + n] = _lin_rows(tm)[2]
            qkv_mem[t, w] = _mem_blocks(mres, s)

        def scores(t):
            qm, km = qkv_mem.pop((t, 0)), qkv_mem.pop((t, 1))
            for n in range(4):
                q = jnp.concatenate([fin[t, 4 * slot + n], qm[n]], 0)
                k = jnp.concatenate([fin[8 + t, 4 * slot + n], km[n], pad], 0).astype(BF16)
                sc = jnp.where(keep, _mm_nt(q, k) * scale, fill)
                e = jnp.exp2(sc - jnp.max(sc, axis=1, keepdims=True))
                probs[t, n] = e, pl.reciprocal(jnp.sum(e, axis=1, keepdims=True), approx=True)

        def values(t):
            vm = qkv_mem.pop((t, 2))
            if s == 0:
                o_old[t] = o_new[t]
            o_mem[t] = []
            for n in range(4):
                v = jnp.concatenate([fin[16 + t, 4 * slot + n], vm[n], pad], 0).astype(BF16)
                e, inv = probs.pop((t, n))
                o = _mm(e, v) * inv
                o_new[t, 4 * s + n] = o[:SEG]
                o_mem[t].append(o[SEG:])

        def out_proj(half, ab):
            lo, hi = span[ab]
            rs = []
            for t in range(4 * half, 4 * half + 4):
                tok = a_side(lambda r, c: o_old[t, 4 * r + c, 8 * lo:8 * hi])(*ab)
                rs.append(_mm(jnp.concatenate([tok, _mem_lhs(*ab, s, o_mem[t])], 0),
                              weight((24 + t) * NPROD + 7 * ab[0] + ab[1])))
            r = (rs[0] + rs[1]) + (rs[2] + rs[3])
            acc[ab] = acc[ab] + r if half else r

        for t in range(8):
            project(t, 0)
            project(t, 1)
            project(t, 2)
            if t:
                values(t - 1)
            scores(t)
        for i, ab in enumerate(prods):
            if i == 8:
                values(7)
            out_proj(0, ab)
        for ab in prods:
            out_proj(1, ab)
        tok, mres = split(acc)
        for (r, n), tm in _token_blocks(tok, outer, inner):
            st = TOUCH[r, n]
            if s != st[0]:
                tm = [(1, (0, 4, yacc[4 * r + n]))] + tm
            val = _lin_rows(tm)[2]
            if s == st[-1]:
                yb[out_rows(jnp.maximum(p - 1, 0), r), lanes(n)] = val.astype(BF16)
            else:
                yacc[4 * r + n] = val
        return tuple(m.astype(BF16).astype(F32) for m in _mem_blocks(mres, s))

    def period(p, mem):
        for s in range(4):
            mem = step(p, s, mem)

        @pl.when(p > 0)
        def _():
            cp_yb(p - 1).start()
        return mem

    m0 = mem0[...].astype(F32)
    last = NSEG // 4 - 1
    lax.fori_loop(0, last + 1, period, tuple(m0[:, lanes(n)] for n in range(4)))

    tok = {}
    for ab in PRODS:
        rs = [_mm(a_side(lambda r, c: o_new[t, 4 * r + c])(*ab), weight((24 + t) * NPROD + 7 * ab[0] + ab[1]))
              for t in range(8)]
        tok[ab] = (0, 4, ((rs[0] + rs[1]) + (rs[2] + rs[3])) + ((rs[4] + rs[5]) + (rs[6] + rs[7])))
    for (r, n), tm in _token_blocks(tok, range(7), range(7)):
        yb[out_rows(last, r), lanes(n)] = _lin_rows(tm)[2].astype(BF16)
    cp_yb(last).start()
    for c in cp_ya:
        c.wait()
    for p in range(last + 1):
        cp_yb(p).wait()


def _run(A_x, A_w_r, A_w_i, B_x, B_mem0, B_Wq, B_Wk, B_Wv, B_Wo):
    vmem = pltpu.VMEM
    out = pl.pallas_call(
        _kernel,
        out_shape=jax.ShapeDtypeStruct((SEQ, 2 * DM), BF16),
        in_specs=[pl.BlockSpec(memory_space=pltpu.HBM)] * 10,
        out_specs=pl.BlockSpec(memory_space=pltpu.HBM),
        scratch_shapes=[
            vmem((4, SEQ // 2, 128), U32), vmem(DFT_CONSTS.shape, U32),
            vmem((16, 128, 128), U32), vmem((16, 128, 128), U32), vmem((2, 1, SEQ), BF16),
            vmem((16, ZROWS, 128), F32), vmem((16, ZROWS, 128), F32), vmem((4, SEQ // 2, 128), U32),
            vmem((SEQ, DM), BF16), vmem((NMEM, DM), BF16),
            vmem((3, DM * HEADS // 2, 128), U32), vmem((4, HEADS * DH // 2, 128), U32),
            vmem((32 * NPROD, 64, 128), U32),
            vmem((16, LEN, 128), F32), vmem((NPROD, SEG, 128), F32),
            vmem((24, 16, SEG, 128), F32), vmem((24, 16, SEG, 128), F32),
            vmem((8, 16, SEG, 128), F32), vmem((8, 16, SEG, 128), F32),
            vmem((16, SEG, 128), F32), vmem((SEQ, DM), BF16),
            pltpu.SemaphoreType.DMA((11,)),
        ],
        compiler_params=pltpu.CompilerParams(vmem_limit_bytes=120 * 2 ** 20),
    )(A_x.reshape(SEQ, DM), A_w_r.T, A_w_i.T, B_x.reshape(SEQ, DM), B_mem0.reshape(NMEM, DM),
      B_Wq.reshape(DM * HEADS, DH), B_Wk.reshape(DM * HEADS, DH), B_Wv.reshape(DM * HEADS, DH),
      B_Wo.reshape(HEADS * DH, DM), DFT_CONSTS)
    return out.reshape(1, SEQ, 2 * DM)


@jax.jit
def pallas_concat_heads__spectral_gfnet__memory_aug_recurrent_mem_tr__prompt_kernel(
    A_x: jax.Array,
    A_w_r: jax.Array,
    A_w_i: jax.Array,
    B_x: jax.Array,
    B_mem0: jax.Array,
    B_Wq: jax.Array,
    B_Wk: jax.Array,
    B_Wv: jax.Array,
    B_Wo: jax.Array,
    B_seg_len: jax.Array,
):
    del B_seg_len
    return _run(A_x, A_w_r, A_w_i, B_x, B_mem0, B_Wq, B_Wk, B_Wv, B_Wo)
```

```python
import itertools

import jax
import jax.numpy as jnp
import numpy as np
from jax import lax
from jax.experimental import pallas as pl
from jax.experimental.pallas import tpu as pltpu

F32, BF16, U32 = jnp.float32, jnp.bfloat16, jnp.uint32
SEQ, DM, HEADS, DH, NMEM, SEG = 2048, 512, 32, 128, 8, 32
NSEG = SEQ // SEG
LEN = NMEM + SEG
LOG2E = 1.4426950408889634

STRASSEN = (
    ({(0, 0): 1, (1, 1): 1}, {(0, 0): 1, (1, 1): 1}, {(0, 0): 1, (1, 1): 1}),
    ({(1, 0): 1, (1, 1): 1}, {(0, 0): 1}, {(1, 0): 1, (1, 1): -1}),
    ({(0, 0): 1}, {(0, 1): 1, (1, 1): -1}, {(0, 1): 1, (1, 1): 1}),
    ({(1, 1): 1}, {(1, 0): 1, (0, 0): -1}, {(0, 0): 1, (1, 0): 1}),
    ({(0, 0): 1, (0, 1): 1}, {(1, 1): 1}, {(0, 0): -1, (0, 1): 1}),
    ({(1, 0): 1, (0, 0): -1}, {(0, 0): 1, (0, 1): 1}, {(1, 1): 1}),
    ({(0, 1): 1, (1, 1): -1}, {(1, 0): 1, (1, 1): 1}, {(0, 0): 1}),
)
PHASE = ((4, 2, 6, 0), (1, 3, 5, 0))
PRODS = tuple(itertools.product(range(7), range(7)))
NPROD = len(PRODS)
LEAD = (3, 2, 1, 0)

STEP_ORDER = ("q0 k0 q1 k1 s0 v0 q2 s1 k2 p0 v1 q3 s2 p1 k3 v2 q4 s3 p2 k4 v3 q5 s4 p3 k5 v4 q6 s5 p4 "
              "k6 v5 q7 s6 p5 k7 v6 w4 s7 p6 v7 x0 w8 p7 w4")
ROW_PATTERN = (4, 2, 4, 2, 4, 2, 4, 2, 4, 2, 4, 2, 4, 4, 1, 4)
EARLY_GROUPS = (0, 8, 1, 9, 16, 2, 10, 17)


def _rows_in_step(a, b, s):
    steps = [2 * p + q for p in range(2) for q in range(2) if a in PHASE[p] and b in PHASE[q]]
    k = steps.index(s)
    return k * 4 // len(steps), (k + 1) * 4 // len(steps)


def _plan(s):
    prods = [(a, b) for a in PHASE[s >> 1] for b in PHASE[s & 1]]
    return prods, {ab: _rows_in_step(*ab, s) for ab in prods}


def _steps_touching(r, n):
    return [s for s in range(4)
            if any((r >> 1, n >> 1) in STRASSEN[a][2] and (r & 1, n & 1) in STRASSEN[b][2] for a, b in _plan(s)[0])]


def _products_without(r):
    return [(a, b) for a, b in PRODS
            if all(any(2 * r1 + r2 != r for r1, _ in STRASSEN[a][k] for r2, _ in STRASSEN[b][k]) for k in (0, 2))]


def _mem_key(a, b, s):
    return tuple(sorted(2 * c1 + c2 for r1, c1 in STRASSEN[a][0] if r1 == s >> 1
                        for r2, c2 in STRASSEN[b][0] if r2 == s & 1))


def _lin(terms):
    terms = sorted(terms, key=lambda t: -t[0])
    c, x = terms[0]
    acc = x if c > 0 else -x
    for c, x in terms[1:]:
        acc = acc + x if c > 0 else acc - x
    return acc


def _lin_rows(terms):
    cuts = sorted({v for _, (lo, hi, _x) in terms for v in (lo, hi)})
    parts = [_lin([(c, x if (l, h) == (lo, hi) else x[8 * (lo - l):8 * (hi - l)])
                   for c, (l, h, x) in terms if l <= lo and hi <= h])
             for lo, hi in zip(cuts[:-1], cuts[1:])]
    return cuts[0], cuts[-1], parts[0] if len(parts) == 1 else jnp.concatenate(parts, 0)


def _inner_blocks(tok, a):
    out = {}
    for rn in itertools.product(range(2), range(2)):
        terms = [(STRASSEN[b][2][rn], tok[a, b]) for b in range(7) if rn in STRASSEN[b][2] and (a, b) in tok]
        if terms:
            out[rn] = _lin_rows(terms)
    return out


def _outer_blocks(mid):
    for r1, n1, r2, n2 in itertools.product(range(2), repeat=4):
        terms = [(STRASSEN[a][2][r1, n1], mid[a][r2, n2]) for a in mid
                 if (r1, n1) in STRASSEN[a][2] and (r2, n2) in mid[a]]
        if terms:
            yield 2 * r1 + r2, 2 * n1 + n2, terms


def _mem_blocks(res, s, ns):
    p, q, mid = s >> 1, s & 1, {}

    def inner(a, n2):
        if (a, n2) not in mid:
            mid[a, n2] = _lin([(STRASSEN[b][2][q, n2], res[a, b]) for b in PHASE[q] if (q, n2) in STRASSEN[b][2]])
        return mid[a, n2]
    return [_lin([(STRASSEN[a][2][p, n >> 1], inner(a, n & 1)) for a in PHASE[p] if (p, n >> 1) in STRASSEN[a][2]])
            for n in ns]


def _left_factors(get, absent=None):
    cache = {}

    def factor(a, b):
        terms = []
        for (r2, c2), cb in STRASSEN[b][0].items():
            if (a, r2, c2) not in cache:
                part = [(ca, get(2 * r1 + r2, 2 * c1 + c2)) for (r1, c1), ca in STRASSEN[a][0].items()
                        if 2 * r1 + r2 != absent]
                cache[a, r2, c2] = _lin(part) if part else None
            if cache[a, r2, c2] is not None:
                terms.append((cb, cache[a, r2, c2]))
        return _lin(terms)
    return factor


def _mm(a, b):
    return jnp.dot(a, b, preferred_element_type=F32)


def _mm_nt(a, b):
    return lax.dot_general(a, b, (((1,), (1,)), ((), ())), preferred_element_type=F32)


def _lo(u):
    return lax.bitcast_convert_type(u << 16, F32)


def _hi(u):
    return lax.bitcast_convert_type(u & np.uint32(0xFFFF0000), F32)


def _pack(both):
    return pltpu.bitcast(both.astype(BF16).reshape(2 * both.shape[0], 128), U32)


def _lanes(c):
    return slice(128 * c, 128 * (c + 1))


def _twiddle(z, k, sign):
    k = (k * sign) % 16
    re, im = z
    if k % 4 == 0:
        return re if k == 0 else -im if k == 4 else -re if k == 8 else im, \
               im if k == 0 else re if k == 4 else -im if k == 8 else -re
    c, s = float(np.cos(np.pi * k / 8)), float(np.sin(np.pi * k / 8))
    if k % 4 == 2:
        return ((re - im) * c, (re + im) * c) if c * s > 0 else ((re + im) * c, (im - re) * c)
    return re * c - im * s, re * s + im * c


def _dft4(z, sign):
    (ar, ai), (br, bi), (cr, ci), (dr, di) = z
    pr, pi, mr, mi = ar + cr, ai + ci, ar - cr, ai - ci
    qr, qi, nr, ni = br + dr, bi + di, br - dr, bi - di
    up, dn = (mr - ni, mi + nr), (mr + ni, mi - nr)
    return [(pr + qr, pi + qi), up if sign > 0 else dn, (pr - qr, pi - qi), dn if sign > 0 else up]


def _dft16(z, sign):
    cols = [_dft4([z[n2 + 4 * n1] for n1 in range(4)], sign) for n2 in range(4)]
    out = [None] * 16
    for k1 in range(4):
        for k2, val in enumerate(_dft4([_twiddle(cols[n2][k1], n2 * k1, sign) for n2 in range(4)], sign)):
            out[k1 + 4 * k2] = val
    return out


def _dft_tables():
    n, k = np.arange(128)[None, :], np.arange(64)[:, None]
    th = [2 * np.pi * ((n * (4 * k + r)) % DM) / DM for r in range(4)]
    c, s = [np.cos(t) for t in th], [np.sin(t) for t in th]
    feat = np.stack([np.concatenate(rows) for rows in (
        (c[0], -s[0]), (c[2], -s[2]), (c[1], -s[1]), (c[3], -s[3]), (-s[1], -c[1]), (s[3], c[3]))])
    feat[0, 64] = np.cos(np.pi * n[0])
    u = feat.astype(np.float32).view(np.uint32)
    h = (u + 0x7FFF + ((u >> 16) & 1)) >> 16
    ph = 2 * np.pi * np.concatenate([(n.T * n) % 128 / 128, np.arange(16)[:, None] * n / SEQ])
    return ((h[:, 0::2] | (h[:, 1::2] << 16)).astype(np.uint32),
            np.stack([np.cos(ph), -np.sin(ph)]).astype(np.float32))


DFT_FEAT, DFT_SEQ = _dft_tables()


def _seq_matrices(table, gmat):
    fr, fi = (jnp.concatenate([table[c, pl.ds(par, 64, stride=2), :] for par in range(2)], 1) for c in range(2))
    norm = 2.0 / (SEQ * DM)
    for a in range(16):
        tr, ti = (jnp.concatenate([table[c, 128 + a:129 + a]] * 2, 1) for c in range(2))
        gr, gi = fr * tr - fi * ti, fr * ti + fi * tr
        for j, g in enumerate((gr, gi - gr, gr + gi, gr * norm, gi * norm)):
            gmat[5 * a + j] = _pack(g)


def _spectral(v, wait_filter, split_code):
    z_re, z_im, tmp = v["z_re"], v["z_im"], v["tmp"]
    sublane = lax.broadcasted_iota(jnp.int32, (8, 128), 0)
    first, never = sublane == 0, sublane < v["zero"][0]
    dmat = lambda i: pltpu.bitcast(v["feat"][i], BF16)
    smat = lambda a, j: pltpu.bitcast(v["gmat"][5 * a + j], BF16)

    for j in range(8):
        words = [v["xa"][c, pl.ds(j, 128, stride=8), :] for c in range(4)]
        for half, unpack in enumerate((_lo, _hi)):
            a = 2 * j + half
            x0, x1, x2, x3 = [unpack(w) for w in words]
            p, q = x0 + x2, x1 + x3
            u, w = (x0 - x2).astype(BF16), (x1 - x3).astype(BF16)
            rs = (_mm_nt(dmat(0), (p + q).astype(BF16)), _mm_nt(dmat(2), u) + _mm_nt(dmat(4), w),
                  _mm_nt(dmat(1), (p - q).astype(BF16)), _mm_nt(dmat(3), u) + _mm_nt(dmat(5), w))
            for r, val in enumerate(rs):
                z_re[a, 8 + 64 * r:72 + 64 * r] = val[:64]
                z_im[a, 8 + 64 * r:72 + 64 * r] = val[64:] if r else jnp.concatenate(
                    [jnp.where(first, 0.0, val[64:72]), val[72:]], 0)
            z_re[a, 0:8] = jnp.where(first, rs[0][64:72], 0.0)

    def forward(r):
        body = slice(8 + 64 * r, 72 + 64 * r)
        rows = body if r else slice(0, 72)
        add = lambda x, y: x + y if r else jnp.concatenate([x[:8], x[8:] + y], 0)
        for a in range(16):
            ure, uim = z_re[a, rows], z_im[a, body]
            both = _mm(add(ure, uim), smat(a, 0))
            z_im[a, rows] = both + _mm(ure, smat(a, 1))
            z_re[a, rows] = val = add(both, -_mm(uim, smat(a, 2)))
            yield val[56:64]

    def inverse(r):
        for a in range(16):
            zr, zi = z_re[a, 8 + 64 * r:72 + 64 * r], z_im[a, 8 + 64 * r:72 + 64 * r]
            bot_r, bot_i = zi, -zr
            if r == 0:
                head = lambda new, old: jnp.concatenate([jnp.where(first, 0.5 * new, old[:8]), old[8:]], 0)
                bot_r, bot_i = head(z_re[a, 0:8], bot_r), head(z_im[a, 0:8], bot_i)
                zr, zi = head(zr[:8], zr), head(zi[:8], zi)
            tmp[4 * a + r] = val = (_mm_nt(smat(a, 3), jnp.concatenate([zr, bot_r], 0).astype(BF16))
                                    + _mm_nt(smat(a, 4), jnp.concatenate([zi, bot_i], 0).astype(BF16)))
            yield val[56:64]

    def mix(row, weight, pace=None):
        z = [(z_re[a, row:row + 8], z_im[a, row:row + 8]) for a in range(16)]
        if pace:
            z[0] = (jnp.where(never, pace[0], z[0][0]), z[0][1])
        y = []
        for k, (xr, xi) in enumerate(_dft16(z, -1)):
            cr, ci = weight(k)
            y.append((xr * cr - xi * ci, xr * ci + xi * cr))
        if pace:
            y[0] = (jnp.where(never, pace[1], y[0][0]), y[0][1])
        for a, (yr, yi) in enumerate(_dft16(y, 1)):
            z_re[a, row:row + 8] = yr
            z_im[a, row:row + 8] = yi

    def apply_filter(r, matmuls):
        if r == 0:
            mix(0, lambda k: tuple(jnp.where(first, v["wnyq"][c, :, _lanes(k)].astype(F32), 0.0) for c in range(2)))
        unpack = (_lo, _hi)[r & 1]
        for blk in range(8):
            src = pl.ds(16 * blk + (r >> 1), 8, stride=2)
            mix(8 + 64 * r + 8 * blk, lambda k: (unpack(v["wr"][k, src, :]), unpack(v["wi"][k, src, :])),
                [next(matmuls), next(matmuls)])

    list(forward(0))
    wait_filter()
    apply_filter(0, forward(1))
    apply_filter(1, forward(2))
    split_code()
    apply_filter(2, forward(3))
    apply_filter(3, inverse(0))
    for r in range(1, 4):
        list(inverse(r))

    for j in range(8):
        u = [[tmp[4 * (2 * j + half) + r] for r in range(4)] for half in range(2)]
        ea = [_mm(x[0], dmat(0)) for x in u]
        eb = [_mm(x[2], dmat(1)) for x in u]
        for c in range(2):
            even = [p - q if c else p + q for p, q in zip(ea, eb)]
            odd = [_mm(x[1], dmat(2 + 2 * c)) + _mm(x[3], dmat(3 + 2 * c)) for x in u]
            v["ya"][c, pl.ds(j, 128, stride=8), :] = _pack(jnp.concatenate([even[0] + odd[0], even[1] + odd[1]], 1))
            v["ya"][c + 2, pl.ds(j, 128, stride=8), :] = _pack(jnp.concatenate([even[0] - odd[0], even[1] - odd[1]], 1))


def _combine_weights(load, wc, base):
    for i in range(8):
        blk = {}
        for a in (0, 1, 4, 2, 5, 3, 6):
            for c1, n1 in STRASSEN[a][1]:
                if (2 * c1, 2 * n1) not in blk:
                    blk.update(load(i, c1, n1))
            mid = {(c2, n2): _lin([(k, blk[2 * c1 + c2, 2 * n1 + n2]) for (c1, n1), k in STRASSEN[a][1].items()])
                   for c2 in range(2) for n2 in range(2)}
            for b in range(7):
                wc[base + 7 * a + b, 8 * i:8 * i + 8, :] = _pack(
                    _lin([(k, mid[cn]) for cn, k in STRASSEN[b][1].items()]))


def _kernel(ax_hbm, wr_hbm, wi_hbm, x_hbm, mem_hbm, wq_hbm, wk_hbm, wv_hbm, wo_hbm, feat_hbm, seq_hbm,
            out_hbm, *scratch):
    v = dict(zip(SCRATCH, scratch))
    xb, yb, wc, sems = v["xb"], v["yb"], v["wc"], v["sems"]
    lhs, part, fin, o_new, o_old, acc, yacc = (v[k] for k in ("lhs", "part", "fin", "o_new", "o_old", "acc", "yacc"))
    copy = pltpu.make_async_copy

    cp_seq = copy(seq_hbm, v["seq"], sems.at[0])
    cp_x0 = copy(x_hbm.at[0:3 * SEG], xb.at[0:3 * SEG], sems.at[1])
    cp_ax = [copy(ax_hbm.bitcast(U32).at[:, _lanes(c)], v["xa"].at[c], sems.at[2]) for c in range(4)]
    cp_ax.append(copy(feat_hbm, v["feat"], sems.at[2]))
    cp_filter = [copy(src.at[0:256].bitcast(U32).at[:, _lanes(k)], dst.at[k], sems.at[3])
                 for src, dst in ((wr_hbm, v["wr"]), (wi_hbm, v["wi"])) for k in range(16)]
    cp_filter += [copy(src.at[256:257, :], v["wnyq"].at[c], sems.at[3]) for c, src in enumerate((wr_hbm, wi_hbm))]
    cp_qkv = [[[copy(src.bitcast(U32).at[:, q, 4 * h:4 * h + 4, :],
                     v["wsrc"].at[8 * w + 2 * h + q % 2, :, 4 * (q // 2):4 * (q // 2) + 4, :], sems.at[4 + 4 * w + h])
                for q in range(4)] for h in range(4)] for w, src in enumerate((wq_hbm, wk_hbm, wv_hbm))]
    cp_wo = [[copy(wo_hbm.bitcast(U32).at[256 * t:256 * t + 256, _lanes(c)],
                   v["wosrc"].at[c, 256 * t:256 * t + 256], sems.at[16 + t]) for c in range(4)] for t in range(8)]
    cp_x1 = [copy(x_hbm.at[3 * SEG:11 * SEG], xb.at[3 * SEG:11 * SEG], sems.at[24]),
             copy(mem_hbm, v["mem0"], sems.at[24])]
    cp_x2 = copy(x_hbm.at[11 * SEG:SEQ], xb.at[11 * SEG:SEQ], sems.at[25])
    cp_ya = [copy(v["ya"].at[c], out_hbm.bitcast(U32).at[:, _lanes(c)], sems.at[26]) for c in range(4)]

    def cp_yb(p):
        return copy(yb.at[pl.ds(pl.multiple_of(p * 128 + 3 * SEG, SEG), 128)],
                    out_hbm.at[pl.ds(pl.multiple_of(p * 128, 128), 128), DM:2 * DM], sems.at[27])

    def start(copies):
        for c in copies:
            c.start()

    def wait(copies):
        for c in copies:
            c.wait()

    start([cp_seq, cp_x0] + cp_ax + cp_filter + sum(cp_qkv[0], []))
    v["zero"][0] = 0

    @pl.loop(0, 2)
    def _(i):
        zero = jnp.zeros((8, 128), F32)
        for k in ("lhs", "yacc", "acc", "ahead", "parked", "tmp", "z_re", "z_im"):
            v[k][i, 0:8] = zero
        for k in ("part", "o_old", "qkv_mem", "o_mem"):
            v[k][i, 0, 0:8] = zero
        v["probs"][i, 0, 0:8] = zero[:, :48]
        v["gmat"][i, 0:8] = lax.bitcast_convert_type(zero, U32)

    weight = lambda g, ab: pltpu.bitcast(wc[g * NPROD + 7 * ab[0] + ab[1]], BF16)

    def x_blocks(seg_of):
        cache = {}

        def get(r, c):
            if r not in cache:
                cache[r] = xb[pl.ds(pl.multiple_of(seg_of(r) * SEG, SEG), SEG), :].astype(F32)
            return cache[r][:, _lanes(c)]
        return get

    for ref in (o_new, acc, yacc):
        ref[...] = jnp.zeros(ref.shape, F32)
    cp_x0.wait()
    first_prods = _products_without(0)
    factor = _left_factors(x_blocks(lambda r: r - 1), absent=0)
    for a, b in first_prods:
        v["lhs0"][7 * a + b] = factor(a, b)
    cp_seq.wait()
    _seq_matrices(v["seq"], v["gmat"])
    wait(cp_ax)

    def wait_filter():
        wait(cp_filter)
        start(sum(cp_qkv[1] + cp_qkv[2], []))

    def split_code():
        @pl.loop(0, 2)
        def _(i):
            v["spare"][i] = jnp.zeros((8, 128), F32)

    _spectral(v, wait_filter, split_code)
    start(cp_x1 + sum(cp_wo, []) + [cp_x2])

    wrows = v["wsrc"].reshape(24, DM * 2, 128)

    def load_qkv(w, t):
        def load(i, c1, n1):
            blk = {}
            for kt in (2 * c1, 2 * c1 + 1):
                rows = pl.ds((64 * kt + 8 * i) * 4 + 2 * (t % 2) + n1, 8, stride=4)
                u = jnp.concatenate([wrows[8 * w + 2 * (t // 2) + par, rows, :] for par in range(2)], 1)
                blk[kt, 2 * n1], blk[kt, 2 * n1 + 1] = _lo(u), _hi(u)
            return blk
        return load

    def load_out(t):
        def load(i, c1, n1):
            blk = {}
            for hd in (2 * c1, 2 * c1 + 1):
                for n in (2 * n1, 2 * n1 + 1):
                    u = v["wosrc"][n, pl.ds((4 * t + hd) * 64 + 8 * i, 8), :]
                    blk[hd, n] = jnp.concatenate([_lo(u), _hi(u)], 1)
            return blk
        return load

    def first_tokens(g):
        seen = set()
        for a in range(7):
            tok = {(a, b): (0, 4, _mm(v["lhs0"][7 * a + b], weight(g, (a, b))))
                   for b in (4, 2, 6, 0, 3, 1, 5) if (a, b) in first_prods}
            for r, n, terms in _outer_blocks({a: _inner_blocks(tok, a)}):
                if r:
                    if (r, n) in seen:
                        terms = [(1, (0, 4, fin[g, 4 * r + n]))] + terms
                    seen.add((r, n))
                    fin[g, 4 * r + n] = _lin_rows(terms)[2]

    arrived = {0: cp_qkv[0], 8: cp_qkv[1], 16: cp_qkv[2][:2], 20: cp_qkv[2][2:],
               24: cp_wo[:2], 26: cp_wo[2:4], 28: cp_wo[4:6], 30: cp_wo[6:7], 31: cp_wo[7:]}
    for g in range(32):
        wait(sum(arrived.get(g, []), []))
        if g >= 8:
            first_tokens(g - 8)
        _combine_weights(load_qkv(g // 8, g % 8) if g < 24 else load_out(g % 8), wc, g * NPROD)
    start(cp_ya)

    row = lax.broadcasted_iota(jnp.int32, (LEN, 48), 0)
    col = lax.broadcasted_iota(jnp.int32, (LEN, 48), 1)
    keep = ((row >= SEG) | (col >= SEG) | (row >= col)) & (col < LEN)
    fill = jnp.where(col < LEN, -1e9 * LOG2E, -jnp.inf).astype(F32)
    scale = DH ** -0.5 * LOG2E
    pad = jnp.zeros((8, 128), F32)

    def out_rows(p, r):
        return pl.ds(pl.multiple_of(p * 128 + r * SEG, SEG), SEG)

    def stage_tokens(p, s):
        prods, span = _plan(s)
        factor = _left_factors(x_blocks(lambda r: jnp.minimum(4 * p + 3 + r, NSEG - 1)))
        for i, ab in enumerate(prods):
            lo, hi = span[ab]
            lhs[i, 0:8 * (hi - lo)] = factor(*ab)[8 * lo:8 * hi]

    def stage_mem(s, mem, which):
        prods, span = _plan(s)
        for i, ab in enumerate(prods):
            if ab in which:
                n = 8 * (span[ab][1] - span[ab][0])
                lhs[i, n:n + 8] = _lin([(1, mem[c]) for c in _mem_key(*ab, s)])

    def lead_products(s):
        return [ab for ab in _plan(s)[0] if (s >> 1, LEAD[s] >> 1) in STRASSEN[ab[0]][2]
                and (s & 1, LEAD[s] & 1) in STRASSEN[ab[1]][2]]

    def new_mem(s, ns):
        prods, span = _plan(s)
        res = {ab: acc[i, 8 * (span[ab][1] - span[ab][0]):8 * (span[ab][1] - span[ab][0]) + 8]
               for i, ab in enumerate(prods) if len(ns) > 1 or ab in lead_products(s)}
        return dict(zip(ns, _mem_blocks(res, s, ns)))

    def emit_tokens(p, s):
        prods, span = _plan(s)
        tok = {ab: (*span[ab], acc[i, 0:8 * (span[ab][1] - span[ab][0])]) for i, ab in enumerate(prods)}
        for r, n, terms in _outer_blocks({a: _inner_blocks(tok, a) for a in PHASE[s >> 1]}):
            steps = _steps_touching(r, n)
            if s != steps[0]:
                terms = [(1, (0, 4, yacc[4 * r + n]))] + terms
            val = _lin_rows(terms)[2]
            if s == steps[-1]:
                yb[out_rows(jnp.maximum(p, 0), r), _lanes(n)] = val.astype(BF16)
            else:
                yacc[4 * r + n] = val

    def step(p, s):
        outer, inner = PHASE[s >> 1], PHASE[s & 1]
        prods, span = _plan(s)
        size = lambda ab: span[ab][1] - span[ab][0]
        prev, nxt = (s - 1) % 4, (s + 1) % 4
        mem_keys = sorted({_mem_key(*ab, s) for ab in prods})
        product = lambda g, ab: _mm(lhs[prods.index(ab), 0:8 * size(ab) + 8], weight(g, ab))

        ready = [ab for ab in prods if _mem_key(*ab, s) == (LEAD[prev],)]
        jobs = [(g, ab) for g in EARLY_GROUPS for ab in sorted(ready, key=lambda ab: -size(ab))[:2]]
        early = {}
        for i in range(0, len(jobs), 4):
            for g, ab in sorted(jobs[i:i + 4], key=lambda job: -size(job[1])):
                early[g, ab] = len(early)
                v["ahead"][early[g, ab], 0:8 * size(ab) + 8] = product(g, ab)
        mem = new_mem(prev, range(4))
        if s == 0:
            mem = {n: jnp.where(p == 0, m0[:, _lanes(n)], mem[n]) for n in range(4)}
        stage_mem(s, mem, [ab for ab in prods if ab not in ready])
        emit_tokens(p - (s == 0), prev)

        def project(g):
            res = {ab: v["ahead"][early[g, ab], 0:8 * size(ab) + 8] if (g, ab) in early else product(g, ab)
                   for ab in prods}
            tok = {ab: (*span[ab], val[:-8]) for ab, val in res.items()}
            mid = {a: _inner_blocks(tok, a) for a in outer}
            for j, (rn, (lo, hi, val)) in enumerate(mid[outer[0]].items()):
                where = (4 * (g % 2) + j, slice(0, 8 * (hi - lo)))
                v["parked"][where] = val
                mid[outer[0]][rn] = (lo, hi, v["parked"][where])
            for r, n, terms in _outer_blocks(mid):
                steps = _steps_touching(r, n)
                if s != steps[0]:
                    terms = [(1, (0, 4, part[g, 4 * r + n]))] + terms
                (fin if s == steps[-1] else part)[g, 4 * r + n] = _lin_rows(terms)[2]
            for n, val in enumerate(_mem_blocks({ab: val[-8:] for ab, val in res.items()}, s, range(4))):
                v["qkv_mem"][g, n] = val

        def rows(g, n):
            return [fin[g, 4 * nxt + n], v["qkv_mem"][g, n]]

        def scores(t):
            for n in range(4):
                q = jnp.concatenate(rows(t, n), 0)
                k = jnp.concatenate(rows(8 + t, n) + [pad], 0).astype(BF16)
                sc = jnp.where(keep, _mm_nt(q, k) * scale, fill)
                e = jnp.exp2(sc - jnp.max(sc, axis=1, keepdims=True))
                v["probs"][t, n] = e * pl.reciprocal(jnp.sum(e, axis=1, keepdims=True), approx=True)

        def values(t):
            if s == 0:
                o_old[t, 0:12] = o_new[t]
            om = []
            for n in range(4):
                o = _mm(v["probs"][t, n], jnp.concatenate(rows(16 + t, n) + [pad], 0).astype(BF16))
                (o_new if s else o_old)[t, 4 * prev + n] = o[:SEG]
                om.append(o[SEG:])
            for i, key in enumerate(mem_keys):
                v["o_mem"][t, i] = _lin([(1, om[c]) for c in key])

        def out_proj(half, ab):
            lo, hi = span[ab]
            rs = []
            for t in range(4 * half, 4 * half + 4):
                tok = _left_factors(lambda r, c: o_old[t, 4 * r + c, 8 * lo:8 * hi])(*ab)
                rs.append(_mm(jnp.concatenate([tok, v["o_mem"][t, mem_keys.index(_mem_key(*ab, s))]], 0),
                              weight(24 + t, ab)))
            total = (rs[0] + rs[1]) + (rs[2] + rs[3])
            where = (prods.index(ab), slice(0, 8 * size(ab) + 8))
            acc[where] = acc[where] + total if half else total

        def alternate(first):
            queue = {n: sorted((ab for ab in prods if size(ab) == n), key=lambda ab: ab not in first)
                     for n in (1, 2, 4)}
            return [queue[n].pop(0) for n in ROW_PATTERN]

        first_half = alternate(())
        for job in STEP_ORDER.split():
            kind, t = job[0], int(job[1:])
            if kind in "qkv":
                project(8 * "qkv".index(kind) + t)
            elif kind == "s":
                scores(t)
            elif kind == "p":
                values(t)
            elif kind == "x":
                xb[SEQ:SEQ + 8, 0:128] = acc[0, 0:8].astype(BF16)
                stage_tokens(p + (s == 3), nxt)
            else:
                for _ in range(t):
                    out_proj(0, first_half.pop(0))
        for i, ab in enumerate(alternate(lead_products(s))):
            out_proj(1, ab)
            if i == 10:
                stage_mem(nxt, new_mem(s, [LEAD[s]]),
                          [ab for ab in _plan(nxt)[0] if _mem_key(*ab, nxt) == (LEAD[s],)])

    wait(cp_x1)
    m0 = v["mem0"][...].astype(F32)
    stage_tokens(0, 0)
    stage_mem(0, [m0[:, _lanes(n)] for n in range(4)], _plan(0)[0])
    last = NSEG // 4 - 1

    @pl.loop(0, last + 1)
    def _(p):
        for s in range(4):
            step(p, s)
        pl.when(p == 0)(cp_x2.wait)
        pl.when(p > 1)(lambda: cp_yb(jnp.maximum(p - 2, 0)).start())

    emit_tokens(last, 3)
    cp_yb(last - 1).start()
    tok = {}
    for ab in _products_without(3):
        rs = [_mm(_left_factors(lambda r, c: o_new[t, 4 * r + c], absent=3)(*ab), weight(24 + t, ab))
              for t in range(8)]
        tok[ab] = (0, 4, ((rs[0] + rs[1]) + (rs[2] + rs[3])) + ((rs[4] + rs[5]) + (rs[6] + rs[7])))
    for r, n, terms in _outer_blocks({a: _inner_blocks(tok, a) for a in range(7)}):
        if r < 3:
            yb[out_rows(last + 1, r), _lanes(n)] = _lin_rows(terms)[2].astype(BF16)
    cp_yb(last).start()
    wait(cp_ya)
    for p in range(last + 1):
        cp_yb(p).wait()


SCRATCH = {
    "xa": ((4, SEQ // 2, 128), U32),
    "feat": (DFT_FEAT.shape, U32),
    "seq": (DFT_SEQ.shape, F32),
    "gmat": ((80, 64, 128), U32),
    "wr": ((16, 128, 128), U32),
    "wi": ((16, 128, 128), U32),
    "wnyq": ((2, 1, SEQ), BF16),
    "z_re": ((16, 264, 128), F32),
    "z_im": ((16, 264, 128), F32),
    "tmp": ((64, 128, 128), F32),
    "ya": ((4, SEQ // 2, 128), U32),
    "xb": ((SEQ + 16, DM), BF16),
    "mem0": ((NMEM, DM), BF16),
    "wsrc": ((24, DM // 4, 8, 128), U32),
    "wosrc": ((4, HEADS * DH // 2, 128), U32),
    "wc": ((32 * NPROD, 64, 128), U32),
    "lhs": ((16, LEN, 128), F32),
    "lhs0": ((NPROD, SEG, 128), F32),
    "part": ((24, 16, SEG, 128), F32),
    "fin": ((24, 16, SEG, 128), F32),
    "o_new": ((8, 12, SEG, 128), F32),
    "o_old": ((8, 16, SEG, 128), F32),
    "yacc": ((16, SEG, 128), F32),
    "yb": ((SEQ + 3 * SEG, DM), BF16),
    "qkv_mem": ((24, 4, 8, 128), F32),
    "probs": ((8, 4, LEN, 48), F32),
    "o_mem": ((8, 9, 8, 128), F32),
    "acc": ((16, LEN, 128), F32),
    "ahead": ((16, LEN, 128), F32),
    "parked": ((8, SEG, 128), F32),
    "spare": ((2, 8, 128), F32),
    "zero": None,
    "sems": None,
}


def _run(A_x, A_w_r, A_w_i, B_x, B_mem0, B_Wq, B_Wk, B_Wv, B_Wo):
    scratch = [pltpu.VMEM(*spec) for spec in SCRATCH.values() if spec]
    out = pl.pallas_call(
        _kernel,
        out_shape=jax.ShapeDtypeStruct((SEQ, 2 * DM), BF16),
        in_specs=[pl.BlockSpec(memory_space=pltpu.HBM)] * 11,
        out_specs=pl.BlockSpec(memory_space=pltpu.HBM),
        scratch_shapes=scratch + [pltpu.SMEM((1,), jnp.int32), pltpu.SemaphoreType.DMA((28,))],
        compiler_params=pltpu.CompilerParams(vmem_limit_bytes=120 * 2 ** 20),
    )(A_x.reshape(SEQ, DM), A_w_r.T, A_w_i.T, B_x.reshape(SEQ, DM), B_mem0.reshape(NMEM, DM),
      *(w.reshape(DM // 4, 4, HEADS, DH) for w in (B_Wq, B_Wk, B_Wv)),
      B_Wo.reshape(HEADS * DH, DM), DFT_FEAT, DFT_SEQ)
    return out.reshape(1, SEQ, 2 * DM)


@jax.jit
def pallas_concat_heads__spectral_gfnet__memory_aug_recurrent_mem_tr__prompt_kernel(
    A_x: jax.Array,
    A_w_r: jax.Array,
    A_w_i: jax.Array,
    B_x: jax.Array,
    B_mem0: jax.Array,
    B_Wq: jax.Array,
    B_Wk: jax.Array,
    B_Wv: jax.Array,
    B_Wo: jax.Array,
    B_seg_len: jax.Array,
):
    del B_seg_len
    return _run(A_x, A_w_r, A_w_i, B_x, B_mem0, B_Wq, B_Wk, B_Wv, B_Wo)
```

```python
import itertools

import jax
import jax.numpy as jnp
import numpy as np
from jax import lax
from jax.experimental import pallas as pl
from jax.experimental.pallas import tpu as pltpu

F32, BF16, U32 = jnp.float32, jnp.bfloat16, jnp.uint32
SEQ, DM, HEADS, DH, NMEM, SEG = 2048, 512, 32, 128, 8, 32
NSEG = SEQ // SEG
LEN = NMEM + SEG
LOG2E = 1.4426950408889634

STRASSEN = (
    ({(0, 0): 1, (1, 1): 1}, {(0, 0): 1, (1, 1): 1}, {(0, 0): 1, (1, 1): 1}),
    ({(1, 0): 1, (1, 1): 1}, {(0, 0): 1}, {(1, 0): 1, (1, 1): -1}),
    ({(0, 0): 1}, {(0, 1): 1, (1, 1): -1}, {(0, 1): 1, (1, 1): 1}),
    ({(1, 1): 1}, {(1, 0): 1, (0, 0): -1}, {(0, 0): 1, (1, 0): 1}),
    ({(0, 0): 1, (0, 1): 1}, {(1, 1): 1}, {(0, 0): -1, (0, 1): 1}),
    ({(1, 0): 1, (0, 0): -1}, {(0, 0): 1, (0, 1): 1}, {(1, 1): 1}),
    ({(0, 1): 1, (1, 1): -1}, {(1, 0): 1, (1, 1): 1}, {(0, 0): 1}),
)
PHASE = ((4, 2, 6, 0), (1, 3, 5, 0))
PRODS = tuple(itertools.product(range(7), range(7)))
NPROD = len(PRODS)
LEAD = (3, 2, 1, 0)

STEP_ORDER = ("k0 q0 k1 q1 s0 v0 k2 s1 q2 p0 v1 k3 s2 p1 q3 v2 k4 s3 p2 q4 v3 k5 s4 p3 q5 v4 k6 s5 p4 "
              "q6 v5 k7 s6 p5 q7 v6 w4 s7 p6 v7 w4 x0 w4 p7 w4")
ROW_PATTERN = (4, 2, 4, 2, 4, 2, 4, 4, 1, 4, 2, 4, 2, 4, 2, 4)
EARLY_GROUPS = (8, 0, 9, 1, 16, 10, 2, 17)


def _rows_in_step(a, b, s):
    steps = [2 * p + q for p in range(2) for q in range(2) if a in PHASE[p] and b in PHASE[q]]
    k = steps.index(s)
    return k * 4 // len(steps), (k + 1) * 4 // len(steps)


def _plan(s):
    prods = [(a, b) for a in PHASE[s >> 1] for b in PHASE[s & 1]]
    return prods, {ab: _rows_in_step(*ab, s) for ab in prods}


def _steps_touching(r, n):
    return [s for s in range(4)
            if any((r >> 1, n >> 1) in STRASSEN[a][2] and (r & 1, n & 1) in STRASSEN[b][2] for a, b in _plan(s)[0])]


def _products_without(r):
    return [(a, b) for a, b in PRODS
            if all(any(2 * r1 + r2 != r for r1, _ in STRASSEN[a][k] for r2, _ in STRASSEN[b][k]) for k in (0, 2))]


def _mem_key(a, b, s):
    return tuple(sorted(2 * c1 + c2 for r1, c1 in STRASSEN[a][0] if r1 == s >> 1
                        for r2, c2 in STRASSEN[b][0] if r2 == s & 1))


def _lin(terms):
    terms = sorted(terms, key=lambda t: -t[0])
    c, x = terms[0]
    acc = x if c > 0 else -x
    for c, x in terms[1:]:
        acc = acc + x if c > 0 else acc - x
    return acc


def _lin_rows(terms):
    cuts = sorted({v for _, (lo, hi, _x) in terms for v in (lo, hi)})
    parts = [_lin([(c, x if (l, h) == (lo, hi) else x[8 * (lo - l):8 * (hi - l)])
                   for c, (l, h, x) in terms if l <= lo and hi <= h])
             for lo, hi in zip(cuts[:-1], cuts[1:])]
    return cuts[0], cuts[-1], parts[0] if len(parts) == 1 else jnp.concatenate(parts, 0)


def _inner_blocks(tok, a):
    out = {}
    for rn in itertools.product(range(2), range(2)):
        terms = [(STRASSEN[b][2][rn], tok[a, b]) for b in range(7) if rn in STRASSEN[b][2] and (a, b) in tok]
        if terms:
            out[rn] = _lin_rows(terms)
    return out


def _outer_blocks(mid):
    for r1, n1, r2, n2 in itertools.product(range(2), repeat=4):
        terms = [(STRASSEN[a][2][r1, n1], mid[a][r2, n2]) for a in mid
                 if (r1, n1) in STRASSEN[a][2] and (r2, n2) in mid[a]]
        if terms:
            yield 2 * r1 + r2, 2 * n1 + n2, terms


def _mem_blocks(res, s, ns):
    p, q, mid = s >> 1, s & 1, {}

    def inner(a, n2):
        if (a, n2) not in mid:
            mid[a, n2] = _lin([(STRASSEN[b][2][q, n2], res[a, b]) for b in PHASE[q] if (q, n2) in STRASSEN[b][2]])
        return mid[a, n2]
    return [_lin([(STRASSEN[a][2][p, n >> 1], inner(a, n & 1)) for a in PHASE[p] if (p, n >> 1) in STRASSEN[a][2]])
            for n in ns]


def _left_factors(get, absent=None):
    cache = {}

    def factor(a, b):
        terms = []
        for (r2, c2), cb in STRASSEN[b][0].items():
            if (a, r2, c2) not in cache:
                part = [(ca, get(2 * r1 + r2, 2 * c1 + c2)) for (r1, c1), ca in STRASSEN[a][0].items()
                        if 2 * r1 + r2 != absent]
                cache[a, r2, c2] = _lin(part) if part else None
            if cache[a, r2, c2] is not None:
                terms.append((cb, cache[a, r2, c2]))
        return _lin(terms)
    return factor


def _mm(a, b):
    return jnp.dot(a, b, preferred_element_type=F32)


def _mm_nt(a, b):
    return lax.dot_general(a, b, (((1,), (1,)), ((), ())), preferred_element_type=F32)


def _lo(u):
    return lax.bitcast_convert_type(u << 16, F32)


def _hi(u):
    return lax.bitcast_convert_type(u & np.uint32(0xFFFF0000), F32)


def _pack(both):
    return pltpu.bitcast(both.astype(BF16).reshape(2 * both.shape[0], 128), U32)


def _lanes(c):
    return slice(128 * c, 128 * (c + 1))


def _twiddle(z, k, sign):
    k = (k * sign) % 16
    re, im = z
    if k == 0:
        return re, im
    if k % 4 == 0:
        return (-im, re) if k == 4 else (-re, -im) if k == 8 else (im, -re)
    c, s = float(np.cos(np.pi * k / 8)), float(np.sin(np.pi * k / 8))
    if k % 4 == 2:
        return ((re - im) * c, (re + im) * c) if c * s > 0 else ((re + im) * c, (im - re) * c)
    return re * c - im * s, re * s + im * c


def _dft4(z, sign):
    (ar, ai), (br, bi), (cr, ci), (dr, di) = z
    pr, pi, mr, mi = ar + cr, ai + ci, ar - cr, ai - ci
    qr, qi, nr, ni = br + dr, bi + di, br - dr, bi - di
    up, dn = (mr - ni, mi + nr), (mr + ni, mi - nr)
    return [(pr + qr, pi + qi), up if sign > 0 else dn, (pr - qr, pi - qi), dn if sign > 0 else up]


def _dft16(z, sign):
    cols = [_dft4([z[n2 + 4 * n1] for n1 in range(4)], sign) for n2 in range(4)]
    out = [None] * 16
    for k1 in range(4):
        for k2, val in enumerate(_dft4([_twiddle(cols[n2][k1], n2 * k1, sign) for n2 in range(4)], sign)):
            out[k1 + 4 * k2] = val
    return out


def _phase_table():
    freq = np.concatenate([np.arange(0, 16, 2) / 128, np.arange(1, 16, 2) / 128, np.arange(8) / 8,
                           np.arange(16) / SEQ])
    angle = 2 * np.pi * freq[:, None] * np.arange(128)[None, :]
    return np.stack([np.cos(angle), -np.sin(angle)]).astype(np.float32)


PHASES = _phase_table()


def _dft_matrices(table, feat, gmat):
    def times(x, row):
        tr, ti = (jnp.concatenate([table[c, row:row + 1]] * 2, 1) for c in range(2))
        return x[0] * tr - x[1] * ti, x[0] * ti + x[1] * tr

    low = [jnp.concatenate([table[c, 0:8], table[c, 8:16]], 1) for c in range(2)]
    base = [jnp.concatenate(part, 0) for part in zip(*(times(low, 16 + i) for i in range(8)))]
    norm = 2.0 / (SEQ * DM)
    for a in range(16):
        gr, gi = times(base, 24 + a)
        for j, g in enumerate((gr, gi - gr, gr + gi, gr * norm, gi * norm)):
            gmat[5 * a + j] = _pack(g)
        cos, nsin = gr[:32], gi[:32]
        if a == 0:
            row, col = (lax.broadcasted_iota(jnp.int32, (32, 256), d) for d in range(2))
            nsin = jnp.where((row == 0) & (col < 128), (1 - 2 * (col & 1)).astype(F32), nsin)
        for j, halves in {0: {0: (cos, nsin)}, 8: {1: (cos, nsin)}, 4: {2: (cos, nsin), 4: (nsin, -cos)},
                          12: {3: (cos, nsin), 5: (-nsin, cos)}}.get(a, {}).items():
            feat[j] = _pack(jnp.concatenate(halves, 0))


def _spectral(v, wait_filter, split_code):
    z_re, z_im, tmp = v["z_re"], v["z_im"], v["tmp"]
    sublane = lax.broadcasted_iota(jnp.int32, (8, 128), 0)
    first, never = sublane == 0, sublane < v["zero"][0]
    dmat = lambda i: pltpu.bitcast(v["feat"][i], BF16)
    smat = lambda a, j: pltpu.bitcast(v["gmat"][5 * a + j], BF16)

    for j in range(8):
        words = [v["xa"][c, pl.ds(j, 128, stride=8), :] for c in range(4)]
        for half, unpack in enumerate((_lo, _hi)):
            a = 2 * j + half
            x0, x1, x2, x3 = [unpack(w) for w in words]
            p, q = x0 + x2, x1 + x3
            u, w = (x0 - x2).astype(BF16), (x1 - x3).astype(BF16)
            rs = (_mm_nt(dmat(0), (p + q).astype(BF16)), _mm_nt(dmat(2), u) + _mm_nt(dmat(4), w),
                  _mm_nt(dmat(1), (p - q).astype(BF16)), _mm_nt(dmat(3), u) + _mm_nt(dmat(5), w))
            for r, val in enumerate(rs):
                z_re[a, 8 + 64 * r:72 + 64 * r] = val[:64]
                z_im[a, 8 + 64 * r:72 + 64 * r] = val[64:] if r else jnp.concatenate(
                    [jnp.where(first, 0.0, val[64:72]), val[72:]], 0)
            z_re[a, 0:8] = jnp.where(first, rs[0][64:72], 0.0)

    def forward(r):
        body = slice(8 + 64 * r, 72 + 64 * r)
        rows = body if r else slice(0, 72)
        add = lambda x, y: x + y if r else jnp.concatenate([x[:8], x[8:] + y], 0)
        for a in range(16):
            ure, uim = z_re[a, rows], z_im[a, body]
            both = _mm(add(ure, uim), smat(a, 0))
            z_im[a, rows] = both + _mm(ure, smat(a, 1))
            z_re[a, rows] = val = add(both, -_mm(uim, smat(a, 2)))
            yield val[56:64]

    def inverse(r):
        for a in range(16):
            zr, zi = z_re[a, 8 + 64 * r:72 + 64 * r], z_im[a, 8 + 64 * r:72 + 64 * r]
            bot_r, bot_i = zi, -zr
            if r == 0:
                head = lambda new, old: jnp.concatenate([jnp.where(first, 0.5 * new, old[:8]), old[8:]], 0)
                bot_r, bot_i = head(z_re[a, 0:8], bot_r), head(z_im[a, 0:8], bot_i)
                zr, zi = head(zr[:8], zr), head(zi[:8], zi)
            tmp[4 * a + r] = val = (_mm_nt(smat(a, 3), jnp.concatenate([zr, bot_r], 0).astype(BF16))
                                    + _mm_nt(smat(a, 4), jnp.concatenate([zi, bot_i], 0).astype(BF16)))
            yield val[56:64]

    def mix(row, weight, pace=None):
        z = [(z_re[a, row:row + 8], z_im[a, row:row + 8]) for a in range(16)]
        if pace:
            z[0] = (jnp.where(never, pace[0], z[0][0]), z[0][1])
        y = []
        for k, (xr, xi) in enumerate(_dft16(z, -1)):
            cr, ci = weight(k)
            y.append((xr * cr - xi * ci, xr * ci + xi * cr))
        if pace:
            y[0] = (jnp.where(never, pace[1], y[0][0]), y[0][1])
        for a, (yr, yi) in enumerate(_dft16(y, 1)):
            z_re[a, row:row + 8] = yr
            z_im[a, row:row + 8] = yi

    def apply_filter(r, matmuls):
        if r == 0:
            mix(0, lambda k: tuple(jnp.where(first, v["wnyq"][c, :, _lanes(k)].astype(F32), 0.0) for c in range(2)))
        unpack = (_lo, _hi)[r & 1]
        for blk in range(8):
            src = pl.ds(16 * blk + (r >> 1), 8, stride=2)
            mix(8 + 64 * r + 8 * blk, lambda k: (unpack(v["wr"][k, src, :]), unpack(v["wi"][k, src, :])),
                [next(matmuls), next(matmuls)])

    list(forward(0))
    wait_filter()
    apply_filter(0, forward(1))
    apply_filter(1, forward(2))
    split_code()
    apply_filter(2, forward(3))
    apply_filter(3, inverse(0))
    for r in range(1, 4):
        list(inverse(r))

    for j in range(8):
        u = [[tmp[4 * (2 * j + half) + r] for r in range(4)] for half in range(2)]
        ea = [_mm(x[0], dmat(0)) for x in u]
        eb = [_mm(x[2], dmat(1)) for x in u]
        for c in range(2):
            even = [p - q if c else p + q for p, q in zip(ea, eb)]
            odd = [_mm(x[1], dmat(2 + 2 * c)) + _mm(x[3], dmat(3 + 2 * c)) for x in u]
            v["ya"][c, pl.ds(j, 128, stride=8), :] = _pack(jnp.concatenate([even[0] + odd[0], even[1] + odd[1]], 1))
            v["ya"][c + 2, pl.ds(j, 128, stride=8), :] = _pack(jnp.concatenate([even[0] - odd[0], even[1] - odd[1]], 1))


def _combine_weights(load, wc, base, matmuls, never):
    issued = [None]
    for i in range(8):
        issued.append(next(matmuls, None))
        pace, blk = issued.pop(0), {}
        for a in (0, 1, 4, 2, 5, 3, 6):
            for c1, n1 in STRASSEN[a][1]:
                if (2 * c1, 2 * n1) not in blk:
                    blk.update(load(i, c1, n1))
                    if pace is not None and (c1, n1) == (1, 0):
                        x = blk[2, 0]
                        blk[2, 0] = jnp.concatenate([jnp.where(never, pace, x[:, :128]), x[:, 128:]], 1)
            mid = {(c2, n2): _lin([(k, blk[2 * c1 + c2, 2 * n1 + n2]) for (c1, n1), k in STRASSEN[a][1].items()])
                   for c2 in range(2) for n2 in range(2)}
            for b in range(7):
                wc[base + 7 * a + b, 8 * i:8 * i + 8, :] = _pack(
                    _lin([(k, mid[cn]) for cn, k in STRASSEN[b][1].items()]))


def _kernel(ax_hbm, wr_hbm, wi_hbm, x_hbm, mem_hbm, wq_hbm, wk_hbm, wv_hbm, wo_hbm, phase_hbm,
            out_hbm, *scratch):
    v = dict(zip(SCRATCH, scratch))
    xb, yb, wc, sems = v["xb"], v["yb"], v["wc"], v["sems"]
    lhs, part, fin, o_new, o_old, acc, yacc = (v[k] for k in ("lhs", "part", "fin", "o_new", "o_old", "acc", "yacc"))
    copy = pltpu.make_async_copy

    cp_phase = copy(phase_hbm, v["phase"], sems.at[0])
    cp_x0 = copy(x_hbm.at[0:3 * SEG], xb.at[0:3 * SEG], sems.at[1])
    cp_ax = [copy(ax_hbm.bitcast(U32).at[:, _lanes(c)], v["xa"].at[c], sems.at[2]) for c in range(4)]
    cp_filter = [copy(src.at[0:256].bitcast(U32).at[:, _lanes(k)], dst.at[k], sems.at[3])
                 for src, dst in ((wr_hbm, v["wr"]), (wi_hbm, v["wi"])) for k in range(16)]
    cp_filter += [copy(src.at[256:257, :], v["wnyq"].at[c], sems.at[3]) for c, src in enumerate((wr_hbm, wi_hbm))]
    cp_qkv = [[[copy(src.bitcast(U32).at[:, q, 4 * h:4 * h + 4, :],
                     v["wsrc"].at[8 * w + 2 * h + q % 2, :, 4 * (q // 2):4 * (q // 2) + 4, :], sems.at[4 + 4 * w + h])
                for q in range(4)] for h in range(4)] for w, src in enumerate((wq_hbm, wk_hbm, wv_hbm))]
    cp_wo = [[copy(wo_hbm.bitcast(U32).at[256 * t:256 * t + 256, _lanes(c)],
                   v["wosrc"].at[c, 256 * t:256 * t + 256], sems.at[16 + t]) for c in range(4)] for t in range(8)]
    cp_x1 = [copy(x_hbm.at[3 * SEG:11 * SEG], xb.at[3 * SEG:11 * SEG], sems.at[24]),
             copy(mem_hbm, v["mem0"], sems.at[24])]
    cp_x2 = copy(x_hbm.at[11 * SEG:SEQ], xb.at[11 * SEG:SEQ], sems.at[25])
    cp_ya = [copy(v["ya"].at[c], out_hbm.bitcast(U32).at[:, _lanes(c)], sems.at[26]) for c in range(4)]

    def cp_yb(p):
        return copy(yb.at[pl.ds(pl.multiple_of(p * 128 + 3 * SEG, SEG), 128)],
                    out_hbm.at[pl.ds(pl.multiple_of(p * 128, 128), 128), DM:2 * DM], sems.at[27])

    def start(copies):
        for c in copies:
            c.start()

    def wait(copies):
        for c in copies:
            c.wait()

    start([cp_phase, cp_x0] + cp_ax + cp_filter + sum(cp_qkv[0], []))
    v["zero"][0] = 0

    @pl.loop(0, 2)
    def _(i):
        zero = jnp.zeros((8, 128), F32)
        for k in ("lhs", "yacc", "acc", "ahead", "parked", "tmp", "z_re", "z_im"):
            v[k][i, 0:8] = zero
        for k in ("part", "o_old", "qkv_mem", "o_mem"):
            v[k][i, 0, 0:8] = zero
        v["probs"][i, 0, 0:8] = zero[:, :48]
        for k in ("gmat", "feat"):
            v[k][i, 0:8] = lax.bitcast_convert_type(zero, U32)

    weight = lambda g, ab: pltpu.bitcast(wc[g * NPROD + 7 * ab[0] + ab[1]], BF16)

    def x_blocks(seg_of):
        cache = {}

        def get(r, c):
            if r not in cache:
                cache[r] = xb[pl.ds(pl.multiple_of(seg_of(r) * SEG, SEG), SEG), :].astype(F32)
            return cache[r][:, _lanes(c)]
        return get

    for ref in (o_new, acc, yacc):
        ref[...] = jnp.zeros(ref.shape, F32)
    cp_x0.wait()
    first_prods = _products_without(0)
    factor = _left_factors(x_blocks(lambda r: r - 1), absent=0)
    for a, b in first_prods:
        v["lhs0"][7 * a + b] = factor(a, b)
    cp_phase.wait()
    _dft_matrices(v["phase"], v["feat"], v["gmat"])
    wait(cp_ax)

    def wait_filter():
        wait(cp_filter)
        start(sum(cp_qkv[1] + cp_qkv[2], []))

    def split_code():
        @pl.loop(0, 2)
        def _(i):
            v["spare"][i] = jnp.zeros((8, 128), F32)

    _spectral(v, wait_filter, split_code)

    wrows = v["wsrc"].reshape(24, DM * 2, 128)

    def load_qkv(w, t):
        def load(i, c1, n1):
            blk = {}
            for kt in (2 * c1, 2 * c1 + 1):
                rows = pl.ds((64 * kt + 8 * i) * 4 + 2 * (t % 2) + n1, 8, stride=4)
                u = jnp.concatenate([wrows[8 * w + 2 * (t // 2) + par, rows, :] for par in range(2)], 1)
                blk[kt, 2 * n1], blk[kt, 2 * n1 + 1] = _lo(u), _hi(u)
            return blk
        return load

    def load_out(t):
        def load(i, c1, n1):
            blk = {}
            for hd in (2 * c1, 2 * c1 + 1):
                for n in (2 * n1, 2 * n1 + 1):
                    u = v["wosrc"][n, pl.ds((4 * t + hd) * 64 + 8 * i, 8), :]
                    blk[hd, n] = jnp.concatenate([_lo(u), _hi(u)], 1)
            return blk
        return load

    def first_tokens(g):
        seen = set()
        for a in range(7):
            tok = {(a, b): (0, 4, _mm(v["lhs0"][7 * a + b], weight(g, (a, b))))
                   for b in (4, 2, 6, 0, 3, 1, 5) if (a, b) in first_prods}
            for r, n, terms in _outer_blocks({a: _inner_blocks(tok, a)}):
                if r:
                    if (r, n) in seen:
                        terms = [(1, (0, 4, fin[g, 4 * r + n]))] + terms
                    seen.add((r, n))
                    fin[g, 4 * r + n] = val = _lin_rows(terms)[2]
            yield val[24:32]

    arrived = {0: cp_qkv[0], 8: cp_qkv[1], 16: cp_qkv[2][:2], 20: cp_qkv[2][2:],
               24: cp_wo[:2], 26: cp_wo[2:4], 28: cp_wo[4:6], 30: cp_wo[6:7], 31: cp_wo[7:]}
    never = lax.broadcasted_iota(jnp.int32, (8, 128), 0) < v["zero"][0]
    for g in range(32):
        if g == 16:
            start(sum(cp_wo, []) + cp_x1)
        if g == 20:
            split_code()
        wait(sum(arrived.get(g, []), []))
        _combine_weights(load_qkv(g // 8, g % 8) if g < 24 else load_out(g % 8), wc, g * NPROD,
                         first_tokens(g - 8) if 8 <= g < 31 else iter(()), never)
        if g == 27:
            list(first_tokens(23))
    start([cp_x2] + cp_ya)

    row = lax.broadcasted_iota(jnp.int32, (LEN, 48), 0)
    col = lax.broadcasted_iota(jnp.int32, (LEN, 48), 1)
    keep = ((row >= SEG) | (col >= SEG) | (row >= col)) & (col < LEN)
    fill = jnp.where(col < LEN, -1e9 * LOG2E, -jnp.inf).astype(F32)
    scale = DH ** -0.5 * LOG2E
    pad = jnp.zeros((8, 128), F32)

    def out_rows(p, r):
        return pl.ds(pl.multiple_of(p * 128 + r * SEG, SEG), SEG)

    def stage_tokens(p, s):
        prods, span = _plan(s)
        factor = _left_factors(x_blocks(lambda r: jnp.minimum(4 * p + 3 + r, NSEG - 1)))
        for i, ab in enumerate(prods):
            lo, hi = span[ab]
            lhs[i, 0:8 * (hi - lo)] = factor(*ab)[8 * lo:8 * hi]

    def stage_mem(s, mem, which):
        prods, span = _plan(s)
        for i, ab in enumerate(prods):
            if ab in which:
                n = 8 * (span[ab][1] - span[ab][0])
                lhs[i, n:n + 8] = _lin([(1, mem[c]) for c in _mem_key(*ab, s)])

    def lead_products(s):
        return [ab for ab in _plan(s)[0] if (s >> 1, LEAD[s] >> 1) in STRASSEN[ab[0]][2]
                and (s & 1, LEAD[s] & 1) in STRASSEN[ab[1]][2]]

    def new_mem(s, ns):
        prods, span = _plan(s)
        res = {ab: acc[i, 8 * (span[ab][1] - span[ab][0]):8 * (span[ab][1] - span[ab][0]) + 8]
               for i, ab in enumerate(prods) if len(ns) > 1 or ab in lead_products(s)}
        return dict(zip(ns, _mem_blocks(res, s, ns)))

    def emit_tokens(p, s):
        prods, span = _plan(s)
        tok = {ab: (*span[ab], acc[i, 0:8 * (span[ab][1] - span[ab][0])]) for i, ab in enumerate(prods)}
        for r, n, terms in _outer_blocks({a: _inner_blocks(tok, a) for a in PHASE[s >> 1]}):
            steps = _steps_touching(r, n)
            if s != steps[0]:
                terms = [(1, (0, 4, yacc[4 * r + n]))] + terms
            val = _lin_rows(terms)[2]
            if s == steps[-1]:
                yb[out_rows(jnp.maximum(p, 0), r), _lanes(n)] = val.astype(BF16)
            else:
                yacc[4 * r + n] = val

    def step(p, s):
        outer, inner = PHASE[s >> 1], PHASE[s & 1]
        prods, span = _plan(s)
        size = lambda ab: span[ab][1] - span[ab][0]
        prev, nxt = (s - 1) % 4, (s + 1) % 4
        mem_keys = sorted({_mem_key(*ab, s) for ab in prods})
        product = lambda g, ab: _mm(lhs[prods.index(ab), 0:8 * size(ab) + 8], weight(g, ab))

        ready = [ab for ab in prods if _mem_key(*ab, s) == (LEAD[prev],)]
        jobs = [(g, ab) for g in EARLY_GROUPS for ab in sorted(ready, key=lambda ab: -size(ab))[:2]]
        early = {}
        for i in range(0, len(jobs), 4):
            for g, ab in sorted(jobs[i:i + 4], key=lambda job: -size(job[1])):
                early[g, ab] = len(early)
                v["ahead"][early[g, ab], 0:8 * size(ab) + 8] = product(g, ab)
        mem = new_mem(prev, range(4))
        if s == 0:
            mem = {n: jnp.where(p == 0, m0[:, _lanes(n)], mem[n]) for n in range(4)}
        stage_mem(s, mem, [ab for ab in prods if ab not in ready])
        emit_tokens(p - (s == 0), prev)

        def project(g):
            res, mid = {}, {}
            for a in outer:
                for b in inner:
                    res[a, b] = (v["ahead"][early[g, (a, b)], 0:8 * size((a, b)) + 8] if (g, (a, b)) in early
                                 else product(g, (a, b)))
                mid[a] = _inner_blocks({(a, b): (*span[a, b], res[a, b][:-8]) for b in inner}, a)
                if a == outer[0]:
                    for j, (rn, (lo, hi, val)) in enumerate(mid[a].items()):
                        where = (4 * (g % 2) + j, slice(0, 8 * (hi - lo)))
                        v["parked"][where] = val
                        mid[a][rn] = (lo, hi, v["parked"][where])
                for r, n, terms in _outer_blocks(mid):
                    if a == [x for x in outer if (r >> 1, n >> 1) in STRASSEN[x][2]][-1]:
                        steps = _steps_touching(r, n)
                        if s != steps[0]:
                            terms = [(1, (0, 4, part[g, 4 * r + n]))] + terms
                        (fin if s == steps[-1] else part)[g, 4 * r + n] = _lin_rows(terms)[2]
            for n, val in enumerate(_mem_blocks({ab: val[-8:] for ab, val in res.items()}, s, range(4))):
                v["qkv_mem"][g, n] = val

        def rows(g, n):
            return [fin[g, 4 * nxt + n], v["qkv_mem"][g, n]]

        def scores(t):
            for n in range(4):
                q = jnp.concatenate(rows(t, n), 0)
                k = jnp.concatenate(rows(8 + t, n) + [pad], 0).astype(BF16)
                sc = jnp.where(keep, _mm_nt(q, k) * scale, fill)
                e = jnp.exp2(sc - jnp.max(sc, axis=1, keepdims=True))
                v["probs"][t, n] = e * pltpu.reciprocal(jnp.sum(e, axis=1, keepdims=True), approx=True)

        def values(t):
            if s == 0:
                o_old[t, 0:12] = o_new[t]
            om = []
            for n in range(4):
                o = _mm(v["probs"][t, n], jnp.concatenate(rows(16 + t, n) + [pad], 0).astype(BF16))
                (o_new if s else o_old)[t, 4 * prev + n] = o[:SEG]
                om.append(o[SEG:])
            for i, key in enumerate(mem_keys):
                v["o_mem"][t, i] = _lin([(1, om[c]) for c in key])

        def out_proj(half, ab):
            lo, hi = span[ab]
            rs = []
            for t in range(4 * half, 4 * half + 4):
                tok = _left_factors(lambda r, c: o_old[t, 4 * r + c, 8 * lo:8 * hi])(*ab)
                rs.append(_mm(jnp.concatenate([tok, v["o_mem"][t, mem_keys.index(_mem_key(*ab, s))]], 0),
                              weight(24 + t, ab)))
            total = (rs[0] + rs[1]) + (rs[2] + rs[3])
            where = (prods.index(ab), slice(0, 8 * size(ab) + 8))
            acc[where] = acc[where] + total if half else total

        def alternate(first):
            queue = {n: sorted((ab for ab in prods if size(ab) == n), key=lambda ab: ab not in first)
                     for n in (1, 2, 4)}
            return [queue[n].pop(0) for n in ROW_PATTERN]

        first_half = alternate(())
        for job in STEP_ORDER.split():
            kind, t = job[0], int(job[1:])
            if kind in "qkv":
                project(8 * "qkv".index(kind) + t)
            elif kind == "s":
                scores(t)
            elif kind == "p":
                values(t)
            elif kind == "x":
                xb[SEQ:SEQ + 8, 0:128] = acc[0, 0:8].astype(BF16)
                stage_tokens(p + (s == 3), nxt)
            else:
                for _ in range(t):
                    out_proj(0, first_half.pop(0))
        for i, ab in enumerate(alternate(lead_products(s))):
            out_proj(1, ab)
            if i == 11:
                stage_mem(nxt, new_mem(s, [LEAD[s]]),
                          [ab for ab in _plan(nxt)[0] if _mem_key(*ab, nxt) == (LEAD[s],)])

    wait(cp_x1)
    m0 = v["mem0"][...].astype(F32)
    stage_tokens(0, 0)
    stage_mem(0, [m0[:, _lanes(n)] for n in range(4)], _plan(0)[0])
    last = NSEG // 4 - 1

    @pl.loop(0, last + 1)
    def _(p):
        for s in range(4):
            step(p, s)
        pl.when(p == 0)(cp_x2.wait)
        pl.when(p > 1)(lambda: cp_yb(jnp.maximum(p - 2, 0)).start())

    emit_tokens(last, 3)
    cp_yb(last - 1).start()
    tok = {}
    for ab in _products_without(3):
        rs = [_mm(_left_factors(lambda r, c: o_new[t, 4 * r + c], absent=3)(*ab), weight(24 + t, ab))
              for t in range(8)]
        tok[ab] = (0, 4, ((rs[0] + rs[1]) + (rs[2] + rs[3])) + ((rs[4] + rs[5]) + (rs[6] + rs[7])))
    for r, n, terms in _outer_blocks({a: _inner_blocks(tok, a) for a in range(7)}):
        if r < 3:
            yb[out_rows(last + 1, r), _lanes(n)] = _lin_rows(terms)[2].astype(BF16)
    cp_yb(last).start()
    wait(cp_ya)
    for p in range(last + 1):
        cp_yb(p).wait()


SCRATCH = {
    "xa": ((4, SEQ // 2, 128), U32),
    "feat": ((6, 64, 128), U32),
    "phase": (PHASES.shape, F32),
    "gmat": ((80, 64, 128), U32),
    "wr": ((16, 128, 128), U32),
    "wi": ((16, 128, 128), U32),
    "wnyq": ((2, 1, SEQ), BF16),
    "z_re": ((16, 264, 128), F32),
    "z_im": ((16, 264, 128), F32),
    "tmp": ((64, 128, 128), F32),
    "ya": ((4, SEQ // 2, 128), U32),
    "xb": ((SEQ + 16, DM), BF16),
    "mem0": ((NMEM, DM), BF16),
    "wsrc": ((24, DM // 4, 8, 128), U32),
    "wosrc": ((4, HEADS * DH // 2, 128), U32),
    "wc": ((32 * NPROD, 64, 128), U32),
    "lhs": ((16, LEN, 128), F32),
    "lhs0": ((NPROD, SEG, 128), F32),
    "part": ((24, 16, SEG, 128), F32),
    "fin": ((24, 16, SEG, 128), F32),
    "o_new": ((8, 12, SEG, 128), F32),
    "o_old": ((8, 16, SEG, 128), F32),
    "yacc": ((16, SEG, 128), F32),
    "yb": ((SEQ + 3 * SEG, DM), BF16),
    "qkv_mem": ((24, 4, 8, 128), F32),
    "probs": ((8, 4, LEN, 48), F32),
    "o_mem": ((8, 9, 8, 128), F32),
    "acc": ((16, LEN, 128), F32),
    "ahead": ((16, LEN, 128), F32),
    "parked": ((8, SEG, 128), F32),
    "spare": ((2, 8, 128), F32),
    "zero": None,
    "sems": None,
}


def _run(A_x, A_w_r, A_w_i, B_x, B_mem0, B_Wq, B_Wk, B_Wv, B_Wo):
    scratch = [pltpu.VMEM(*spec) for spec in SCRATCH.values() if spec]
    out = pl.pallas_call(
        _kernel,
        out_shape=jax.ShapeDtypeStruct((SEQ, 2 * DM), BF16),
        in_specs=[pl.BlockSpec(memory_space=pltpu.HBM)] * 10,
        out_specs=pl.BlockSpec(memory_space=pltpu.HBM),
        scratch_shapes=scratch + [pltpu.SMEM((1,), jnp.int32), pltpu.SemaphoreType.DMA((28,))],
        compiler_params=pltpu.CompilerParams(vmem_limit_bytes=120 * 2 ** 20),
    )(A_x.reshape(SEQ, DM), A_w_r.T, A_w_i.T, B_x.reshape(SEQ, DM), B_mem0.reshape(NMEM, DM),
      *(w.reshape(DM // 4, 4, HEADS, DH) for w in (B_Wq, B_Wk, B_Wv)),
      B_Wo.reshape(HEADS * DH, DM), PHASES)
    return out.reshape(1, SEQ, 2 * DM)


@jax.jit
def pallas_concat_heads__spectral_gfnet__memory_aug_recurrent_mem_tr__prompt_kernel(
    A_x: jax.Array,
    A_w_r: jax.Array,
    A_w_i: jax.Array,
    B_x: jax.Array,
    B_mem0: jax.Array,
    B_Wq: jax.Array,
    B_Wk: jax.Array,
    B_Wv: jax.Array,
    B_Wo: jax.Array,
    B_seg_len: jax.Array,
):
    del B_seg_len
    return _run(A_x, A_w_r, A_w_i, B_x, B_mem0, B_Wq, B_Wk, B_Wv, B_Wo)
```

```python
import itertools

import jax
import jax.numpy as jnp
import numpy as np
from jax import lax
from jax.experimental import pallas as pl
from jax.experimental.pallas import tpu as pltpu

F32, BF16, U32 = jnp.float32, jnp.bfloat16, jnp.uint32
SEQ, DM, HEADS, DH, NMEM, SEG = 2048, 512, 32, 128, 8, 32
NSEG = SEQ // SEG
LEN = NMEM + SEG
LOG2E = 1.4426950408889634

STRASSEN = (
    ({(0, 0): 1, (1, 1): 1}, {(0, 0): 1, (1, 1): 1}, {(0, 0): 1, (1, 1): 1}),
    ({(1, 0): 1, (1, 1): 1}, {(0, 0): 1}, {(1, 0): 1, (1, 1): -1}),
    ({(0, 0): 1}, {(0, 1): 1, (1, 1): -1}, {(0, 1): 1, (1, 1): 1}),
    ({(1, 1): 1}, {(1, 0): 1, (0, 0): -1}, {(0, 0): 1, (1, 0): 1}),
    ({(0, 0): 1, (0, 1): 1}, {(1, 1): 1}, {(0, 0): -1, (0, 1): 1}),
    ({(1, 0): 1, (0, 0): -1}, {(0, 0): 1, (0, 1): 1}, {(1, 1): 1}),
    ({(0, 1): 1, (1, 1): -1}, {(1, 0): 1, (1, 1): 1}, {(0, 0): 1}),
)
PHASE = ((4, 2, 6, 0), (1, 3, 5, 0))
PRODS = tuple(itertools.product(range(7), range(7)))
NPROD = len(PRODS)
LEAD = (3, 2, 1, 0)

STEP_ORDER = ("k0 q0 k1 q1 s0 v0 k2 s1 q2 p0 v1 k3 s2 p1 q3 v2 k4 s3 p2 q4 v3 k5 s4 p3 q5 v4 k6 s5 p4 "
              "q6 v5 k7 s6 p5 q7 v6 w4 s7 p6 v7 w4 x0 w4 p7 w4")
ROW_PATTERN = (4, 2, 4, 2, 4, 2, 4, 4, 1, 4, 2, 4, 2, 4, 2, 4)
EARLY_GROUPS = (8, 0, 9, 1, 16, 10, 2, 17)


def _rows_in_step(a, b, s):
    steps = [2 * p + q for p in range(2) for q in range(2) if a in PHASE[p] and b in PHASE[q]]
    k = steps.index(s)
    return k * 4 // len(steps), (k + 1) * 4 // len(steps)


def _plan(s):
    prods = [(a, b) for a in PHASE[s >> 1] for b in PHASE[s & 1]]
    return prods, {ab: _rows_in_step(*ab, s) for ab in prods}


def _steps_touching(r, n):
    return [s for s in range(4)
            if any((r >> 1, n >> 1) in STRASSEN[a][2] and (r & 1, n & 1) in STRASSEN[b][2] for a, b in _plan(s)[0])]


def _products_without(r):
    return [(a, b) for a, b in PRODS
            if all(any(2 * r1 + r2 != r for r1, _ in STRASSEN[a][k] for r2, _ in STRASSEN[b][k]) for k in (0, 2))]


def _mem_key(a, b, s):
    return tuple(sorted(2 * c1 + c2 for r1, c1 in STRASSEN[a][0] if r1 == s >> 1
                        for r2, c2 in STRASSEN[b][0] if r2 == s & 1))


def _lin(terms):
    terms = sorted(terms, key=lambda t: -t[0])
    c, x = terms[0]
    acc = x if c > 0 else -x
    for c, x in terms[1:]:
        acc = acc + x if c > 0 else acc - x
    return acc


def _lin_rows(terms):
    cuts = sorted({v for _, (lo, hi, _x) in terms for v in (lo, hi)})
    parts = [_lin([(c, x if (l, h) == (lo, hi) else x[8 * (lo - l):8 * (hi - l)])
                   for c, (l, h, x) in terms if l <= lo and hi <= h])
             for lo, hi in zip(cuts[:-1], cuts[1:])]
    return cuts[0], cuts[-1], parts[0] if len(parts) == 1 else jnp.concatenate(parts, 0)


def _inner_blocks(tok, a):
    out = {}
    for rn in itertools.product(range(2), range(2)):
        terms = [(STRASSEN[b][2][rn], tok[a, b]) for b in range(7) if rn in STRASSEN[b][2] and (a, b) in tok]
        if terms:
            out[rn] = _lin_rows(terms)
    return out


def _outer_blocks(mid):
    for r1, n1, r2, n2 in itertools.product(range(2), repeat=4):
        terms = [(STRASSEN[a][2][r1, n1], mid[a][r2, n2]) for a in mid
                 if (r1, n1) in STRASSEN[a][2] and (r2, n2) in mid[a]]
        if terms:
            yield 2 * r1 + r2, 2 * n1 + n2, terms


def _mem_blocks(res, s, ns):
    p, q, mid = s >> 1, s & 1, {}

    def inner(a, n2):
        if (a, n2) not in mid:
            mid[a, n2] = _lin([(STRASSEN[b][2][q, n2], res[a, b]) for b in PHASE[q] if (q, n2) in STRASSEN[b][2]])
        return mid[a, n2]
    return [_lin([(STRASSEN[a][2][p, n >> 1], inner(a, n & 1)) for a in PHASE[p] if (p, n >> 1) in STRASSEN[a][2]])
            for n in ns]


def _left_factors(get, absent=None):
    cache = {}

    def factor(a, b):
        terms = []
        for (r2, c2), cb in STRASSEN[b][0].items():
            if (a, r2, c2) not in cache:
                part = [(ca, get(2 * r1 + r2, 2 * c1 + c2)) for (r1, c1), ca in STRASSEN[a][0].items()
                        if 2 * r1 + r2 != absent]
                cache[a, r2, c2] = _lin(part) if part else None
            if cache[a, r2, c2] is not None:
                terms.append((cb, cache[a, r2, c2]))
        return _lin(terms)
    return factor


def _mm(a, b):
    return jnp.dot(a, b, preferred_element_type=F32)


def _mm_nt(a, b):
    return lax.dot_general(a, b, (((1,), (1,)), ((), ())), preferred_element_type=F32)


def _lo(u):
    return lax.bitcast_convert_type(u << 16, F32)


def _hi(u):
    return lax.bitcast_convert_type(u & np.uint32(0xFFFF0000), F32)


def _pack(both):
    return pltpu.bitcast(both.astype(BF16).reshape(2 * both.shape[0], 128), U32)


def _lanes(c):
    return slice(128 * c, 128 * (c + 1))


def _twiddle(z, k, sign):
    k = (k * sign) % 16
    re, im = z
    if k == 0:
        return re, im
    if k % 4 == 0:
        return (-im, re) if k == 4 else (-re, -im) if k == 8 else (im, -re)
    c, s = float(np.cos(np.pi * k / 8)), float(np.sin(np.pi * k / 8))
    if k % 4 == 2:
        return ((re - im) * c, (re + im) * c) if c * s > 0 else ((re + im) * c, (im - re) * c)
    return re * c - im * s, re * s + im * c


def _dft4(z, sign):
    (ar, ai), (br, bi), (cr, ci), (dr, di) = z
    pr, pi, mr, mi = ar + cr, ai + ci, ar - cr, ai - ci
    qr, qi, nr, ni = br + dr, bi + di, br - dr, bi - di
    up, dn = (mr - ni, mi + nr), (mr + ni, mi - nr)
    return [(pr + qr, pi + qi), up if sign > 0 else dn, (pr - qr, pi - qi), dn if sign > 0 else up]


def _dft16(z, sign):
    cols = [_dft4([z[n2 + 4 * n1] for n1 in range(4)], sign) for n2 in range(4)]
    out = [None] * 16
    for k1 in range(4):
        for k2, val in enumerate(_dft4([_twiddle(cols[n2][k1], n2 * k1, sign) for n2 in range(4)], sign)):
            out[k1 + 4 * k2] = val
    return out


def _phase_table():
    freq = np.concatenate([np.arange(0, 16, 2) / 128, np.arange(1, 16, 2) / 128, np.arange(8) / 8,
                           np.arange(16) / SEQ])
    angle = 2 * np.pi * freq[:, None] * np.arange(128)[None, :]
    return np.stack([np.cos(angle), -np.sin(angle)]).astype(np.float32)


PHASES = _phase_table()


def _dft_matrices(table, feat, gmat):
    def times(x, row):
        tr, ti = (jnp.concatenate([table[c, row:row + 1]] * 2, 1) for c in range(2))
        return x[0] * tr - x[1] * ti, x[0] * ti + x[1] * tr

    low = [jnp.concatenate([table[c, 0:8], table[c, 8:16]], 1) for c in range(2)]
    base = [jnp.concatenate(part, 0) for part in zip(*(times(low, 16 + i) for i in range(8)))]
    norm = 2.0 / (SEQ * DM)
    for a in range(16):
        gr, gi = times(base, 24 + a)
        for j, g in enumerate((gr, gi - gr, gr + gi, gr * norm, gi * norm)):
            gmat[5 * a + j] = _pack(g)
        cos, nsin = gr[:32], gi[:32]
        if a == 0:
            row, col = (lax.broadcasted_iota(jnp.int32, (32, 256), d) for d in range(2))
            nsin = jnp.where((row == 0) & (col < 128), (1 - 2 * (col & 1)).astype(F32), nsin)
        for j, halves in {0: {0: (cos, nsin)}, 8: {1: (cos, nsin)}, 4: {2: (cos, nsin), 4: (nsin, -cos)},
                          12: {3: (cos, nsin), 5: (-nsin, cos)}}.get(a, {}).items():
            feat[j] = _pack(jnp.concatenate(halves, 0))


def _spectral(v, wait_filter, split_code):
    z_re, z_im, tmp = v["z_re"], v["z_im"], v["tmp"]
    sublane = lax.broadcasted_iota(jnp.int32, (8, 128), 0)
    first, never = sublane == 0, sublane < v["zero"][0]
    dmat = lambda i: pltpu.bitcast(v["feat"][i], BF16)
    smat = lambda a, j: pltpu.bitcast(v["gmat"][5 * a + j], BF16)

    for j in range(8):
        words = [v["xa"][c, pl.ds(j, 128, stride=8), :] for c in range(4)]
        for half, unpack in enumerate((_lo, _hi)):
            a = 2 * j + half
            x0, x1, x2, x3 = [unpack(w) for w in words]
            p, q = x0 + x2, x1 + x3
            u, w = (x0 - x2).astype(BF16), (x1 - x3).astype(BF16)
            rs = (_mm_nt(dmat(0), (p + q).astype(BF16)), _mm_nt(dmat(2), u) + _mm_nt(dmat(4), w),
                  _mm_nt(dmat(1), (p - q).astype(BF16)), _mm_nt(dmat(3), u) + _mm_nt(dmat(5), w))
            for r, val in enumerate(rs):
                z_re[a, 8 + 64 * r:72 + 64 * r] = val[:64]
                z_im[a, 8 + 64 * r:72 + 64 * r] = val[64:] if r else jnp.concatenate(
                    [jnp.where(first, 0.0, val[64:72]), val[72:]], 0)
            z_re[a, 0:8] = jnp.where(first, rs[0][64:72], 0.0)

    def forward(r):
        body = slice(8 + 64 * r, 72 + 64 * r)
        rows = body if r else slice(0, 72)
        add = lambda x, y: x + y if r else jnp.concatenate([x[:8], x[8:] + y], 0)
        for a in range(16):
            ure, uim = z_re[a, rows], z_im[a, body]
            both = _mm(add(ure, uim), smat(a, 0))
            z_im[a, rows] = both + _mm(ure, smat(a, 1))
            z_re[a, rows] = val = add(both, -_mm(uim, smat(a, 2)))
            yield val[56:64]

    def inverse(r):
        for a in range(16):
            zr, zi = z_re[a, 8 + 64 * r:72 + 64 * r], z_im[a, 8 + 64 * r:72 + 64 * r]
            bot_r, bot_i = zi, -zr
            if r == 0:
                head = lambda new, old: jnp.concatenate([jnp.where(first, 0.5 * new, old[:8]), old[8:]], 0)
                bot_r, bot_i = head(z_re[a, 0:8], bot_r), head(z_im[a, 0:8], bot_i)
                zr, zi = head(zr[:8], zr), head(zi[:8], zi)
            tmp[4 * a + r] = val = (_mm_nt(smat(a, 3), jnp.concatenate([zr, bot_r], 0).astype(BF16))
                                    + _mm_nt(smat(a, 4), jnp.concatenate([zi, bot_i], 0).astype(BF16)))
            yield val[56:64]

    def mix(row, weight, pace=None):
        z = [(z_re[a, row:row + 8], z_im[a, row:row + 8]) for a in range(16)]
        if pace:
            z[0] = (jnp.where(never, pace[0], z[0][0]), z[0][1])
        y = []
        for k, (xr, xi) in enumerate(_dft16(z, -1)):
            cr, ci = weight(k)
            y.append((xr * cr - xi * ci, xr * ci + xi * cr))
        if pace:
            y[0] = (jnp.where(never, pace[1], y[0][0]), y[0][1])
        for a, (yr, yi) in enumerate(_dft16(y, 1)):
            z_re[a, row:row + 8] = yr
            z_im[a, row:row + 8] = yi

    def apply_filter(r, matmuls):
        if r == 0:
            mix(0, lambda k: tuple(jnp.where(first, v["wnyq"][c, :, _lanes(k)].astype(F32), 0.0) for c in range(2)))
        unpack = (_lo, _hi)[r & 1]
        for blk in range(8):
            src = pl.ds(16 * blk + (r >> 1), 8, stride=2)
            mix(8 + 64 * r + 8 * blk, lambda k: (unpack(v["wr"][k, src, :]), unpack(v["wi"][k, src, :])),
                [next(matmuls), next(matmuls)])

    list(forward(0))
    wait_filter()
    apply_filter(0, forward(1))
    apply_filter(1, forward(2))
    split_code()
    apply_filter(2, forward(3))
    apply_filter(3, inverse(0))
    for r in range(1, 4):
        list(inverse(r))

    for j in range(8):
        u = [[tmp[4 * (2 * j + half) + r] for r in range(4)] for half in range(2)]
        ea = [_mm(x[0], dmat(0)) for x in u]
        eb = [_mm(x[2], dmat(1)) for x in u]
        for c in range(2):
            even = [p - q if c else p + q for p, q in zip(ea, eb)]
            odd = [_mm(x[1], dmat(2 + 2 * c)) + _mm(x[3], dmat(3 + 2 * c)) for x in u]
            v["ya"][c, pl.ds(j, 128, stride=8), :] = _pack(jnp.concatenate([even[0] + odd[0], even[1] + odd[1]], 1))
            v["ya"][c + 2, pl.ds(j, 128, stride=8), :] = _pack(jnp.concatenate([even[0] - odd[0], even[1] - odd[1]], 1))


def _combine_weights(load, wc, base, matmuls, never):
    issued = [None]
    for i in range(8):
        issued.append(next(matmuls, None))
        pace, blk = issued.pop(0), {}
        for a in (0, 1, 4, 2, 5, 3, 6):
            for c1, n1 in STRASSEN[a][1]:
                if (2 * c1, 2 * n1) not in blk:
                    blk.update(load(i, c1, n1))
                    if pace is not None and (c1, n1) == (1, 0):
                        x = blk[2, 0]
                        blk[2, 0] = jnp.concatenate([jnp.where(never, pace, x[:, :128]), x[:, 128:]], 1)
            mid = {(c2, n2): _lin([(k, blk[2 * c1 + c2, 2 * n1 + n2]) for (c1, n1), k in STRASSEN[a][1].items()])
                   for c2 in range(2) for n2 in range(2)}
            for b in range(7):
                wc[base + 7 * a + b, 8 * i:8 * i + 8, :] = _pack(
                    _lin([(k, mid[cn]) for cn, k in STRASSEN[b][1].items()]))


def _kernel(ax_hbm, wr_hbm, wi_hbm, x_hbm, mem_hbm, wq_hbm, wk_hbm, wv_hbm, wo_hbm, phase_hbm,
            out_hbm, *scratch):
    v = dict(zip(SCRATCH, scratch))
    xb, yb, wc, sems = v["xb"], v["yb"], v["wc"], v["sems"]
    lhs, part, fin, o_new, o_old, acc, yacc = (v[k] for k in ("lhs", "part", "fin", "o_new", "o_old", "acc", "yacc"))
    copy = pltpu.make_async_copy

    cp_phase = copy(phase_hbm, v["phase"], sems.at[0])
    cp_x0 = copy(x_hbm.at[0:3 * SEG], xb.at[0:3 * SEG], sems.at[1])
    cp_ax = [copy(ax_hbm.bitcast(U32).at[:, _lanes(c)], v["xa"].at[c], sems.at[2]) for c in range(4)]
    cp_filter = [copy(src.at[0:256].bitcast(U32).at[:, _lanes(k)], dst.at[k], sems.at[3])
                 for src, dst in ((wr_hbm, v["wr"]), (wi_hbm, v["wi"])) for k in range(16)]
    cp_filter += [copy(src.at[256:257, :], v["wnyq"].at[c], sems.at[3]) for c, src in enumerate((wr_hbm, wi_hbm))]
    cp_qkv = [[[copy(src.bitcast(U32).at[:, q, 4 * h:4 * h + 4, :],
                     v["wsrc"].at[8 * w + 2 * h + q % 2, :, 4 * (q // 2):4 * (q // 2) + 4, :], sems.at[4 + 4 * w + h])
                for q in range(4)] for h in range(4)] for w, src in enumerate((wq_hbm, wk_hbm, wv_hbm))]
    cp_wo = [[copy(wo_hbm.bitcast(U32).at[256 * t:256 * t + 256, _lanes(c)],
                   v["wosrc"].at[c, 256 * t:256 * t + 256], sems.at[16 + t]) for c in range(4)] for t in range(8)]
    cp_x1 = [copy(x_hbm.at[3 * SEG:11 * SEG], xb.at[3 * SEG:11 * SEG], sems.at[24]),
             copy(mem_hbm, v["mem0"], sems.at[24])]
    cp_x2 = copy(x_hbm.at[11 * SEG:SEQ], xb.at[11 * SEG:SEQ], sems.at[25])
    cp_ya = [copy(v["ya"].at[c], out_hbm.bitcast(U32).at[:, _lanes(c)], sems.at[26]) for c in range(4)]

    def cp_yb(p):
        return copy(yb.at[pl.ds(pl.multiple_of(p * 128 + 3 * SEG, SEG), 128)],
                    out_hbm.at[pl.ds(pl.multiple_of(p * 128, 128), 128), DM:2 * DM], sems.at[27])

    def start(copies):
        for c in copies:
            c.start()

    def wait(copies):
        for c in copies:
            c.wait()

    start([cp_phase, cp_x0] + cp_ax + cp_filter + sum(cp_qkv[0], []))
    v["zero"][0] = 0

    @pl.loop(0, 2)
    def _(i):
        zero = jnp.zeros((8, 128), F32)
        for k in ("lhs", "yacc", "acc", "ahead", "parked", "tmp", "z_re", "z_im"):
            v[k][i, 0:8] = zero
        for k in ("part", "o_old", "qkv_mem", "o_mem"):
            v[k][i, 0, 0:8] = zero
        v["probs"][i, 0, 0:8] = zero[:, :48]
        for k in ("gmat", "feat"):
            v[k][i, 0:8] = lax.bitcast_convert_type(zero, U32)

    weight = lambda g, ab: pltpu.bitcast(wc[g * NPROD + 7 * ab[0] + ab[1]], BF16)

    def x_blocks(seg_of):
        cache = {}

        def get(r, c):
            if r not in cache:
                cache[r] = xb[pl.ds(pl.multiple_of(seg_of(r) * SEG, SEG), SEG), :].astype(F32)
            return cache[r][:, _lanes(c)]
        return get

    o_new[...] = jnp.zeros(o_new.shape, F32)
    cp_x0.wait()
    first_prods = _products_without(0)
    factor = _left_factors(x_blocks(lambda r: r - 1), absent=0)
    for a, b in first_prods:
        v["lhs0"][7 * a + b] = factor(a, b)
    cp_phase.wait()
    _dft_matrices(v["phase"], v["feat"], v["gmat"])
    wait(cp_ax)

    def wait_filter():
        wait(cp_filter)
        start(sum(cp_qkv[1] + cp_qkv[2], []))

    def split_code():
        @pl.loop(0, 2)
        def _(i):
            v["spare"][i] = jnp.zeros((8, 128), F32)

    _spectral(v, wait_filter, split_code)

    wrows = v["wsrc"].reshape(24, DM * 2, 128)

    def load_qkv(w, t):
        def load(i, c1, n1):
            blk = {}
            for kt in (2 * c1, 2 * c1 + 1):
                rows = pl.ds((64 * kt + 8 * i) * 4 + 2 * (t % 2) + n1, 8, stride=4)
                u = jnp.concatenate([wrows[8 * w + 2 * (t // 2) + par, rows, :] for par in range(2)], 1)
                blk[kt, 2 * n1], blk[kt, 2 * n1 + 1] = _lo(u), _hi(u)
            return blk
        return load

    def load_out(t):
        def load(i, c1, n1):
            blk = {}
            for hd in (2 * c1, 2 * c1 + 1):
                for n in (2 * n1, 2 * n1 + 1):
                    u = v["wosrc"][n, pl.ds((4 * t + hd) * 64 + 8 * i, 8), :]
                    blk[hd, n] = jnp.concatenate([_lo(u), _hi(u)], 1)
            return blk
        return load

    def first_tokens(g):
        seen = set()
        for a in range(7):
            tok = {(a, b): (0, 4, _mm(v["lhs0"][7 * a + b], weight(g, (a, b))))
                   for b in (4, 2, 6, 0, 3, 1, 5) if (a, b) in first_prods}
            for r, n, terms in _outer_blocks({a: _inner_blocks(tok, a)}):
                if r:
                    if (r, n) in seen:
                        terms = [(1, (0, 4, fin[g, 4 * r + n]))] + terms
                    seen.add((r, n))
                    fin[g, 4 * r + n] = val = _lin_rows(terms)[2]
            yield val[24:32]

    arrived = {0: cp_qkv[0], 8: cp_qkv[1], 16: cp_qkv[2][:2], 20: cp_qkv[2][2:],
               24: cp_wo[:2], 26: cp_wo[2:4], 28: cp_wo[4:6], 30: cp_wo[6:7], 31: cp_wo[7:]}
    never = lax.broadcasted_iota(jnp.int32, (8, 128), 0) < v["zero"][0]
    for g in range(32):
        if g == 16:
            start(sum(cp_wo, []) + cp_x1)
        if g == 20:
            split_code()
        wait(sum(arrived.get(g, []), []))
        _combine_weights(load_qkv(g // 8, g % 8) if g < 24 else load_out(g % 8), wc, g * NPROD,
                         first_tokens(g - 8) if 8 <= g < 31 else iter(()), never)
        if g == 27:
            list(first_tokens(23))
    start([cp_x2] + cp_ya)

    row = lax.broadcasted_iota(jnp.int32, (LEN, 48), 0)
    col = lax.broadcasted_iota(jnp.int32, (LEN, 48), 1)
    keep = ((row >= SEG) | (col >= SEG) | (row >= col)) & (col < LEN)
    fill = jnp.where(col < LEN, -1e9 * LOG2E, -jnp.inf).astype(F32)
    scale = DH ** -0.5 * LOG2E
    pad = jnp.zeros((8, 128), F32)

    def out_rows(p, r):
        return pl.ds(pl.multiple_of(p * 128 + r * SEG, SEG), SEG)

    def stage_tokens(p, s):
        prods, span = _plan(s)
        factor = _left_factors(x_blocks(lambda r: jnp.minimum(4 * p + 3 + r, NSEG - 1)))
        for i, ab in enumerate(prods):
            lo, hi = span[ab]
            lhs[i, 0:8 * (hi - lo)] = factor(*ab)[8 * lo:8 * hi]

    def stage_mem(s, mem, which):
        prods, span = _plan(s)
        for i, ab in enumerate(prods):
            if ab in which:
                n = 8 * (span[ab][1] - span[ab][0])
                lhs[i, n:n + 8] = _lin([(1, mem[c]) for c in _mem_key(*ab, s)])

    def lead_products(s):
        return [ab for ab in _plan(s)[0] if (s >> 1, LEAD[s] >> 1) in STRASSEN[ab[0]][2]
                and (s & 1, LEAD[s] & 1) in STRASSEN[ab[1]][2]]

    def new_mem(s, ns):
        prods, span = _plan(s)
        res = {ab: acc[i, 8 * (span[ab][1] - span[ab][0]):8 * (span[ab][1] - span[ab][0]) + 8]
               for i, ab in enumerate(prods) if len(ns) > 1 or ab in lead_products(s)}
        return dict(zip(ns, _mem_blocks(res, s, ns)))

    def emit_tokens(p, s):
        prods, span = _plan(s)
        tok = {ab: (*span[ab], acc[i, 0:8 * (span[ab][1] - span[ab][0])]) for i, ab in enumerate(prods)}
        for r, n, terms in _outer_blocks({a: _inner_blocks(tok, a) for a in PHASE[s >> 1]}):
            steps = _steps_touching(r, n)
            if s != steps[0]:
                terms = [(1, (0, 4, yacc[4 * r + n]))] + terms
            val = _lin_rows(terms)[2]
            if s == steps[-1]:
                yb[out_rows(p, r), _lanes(n)] = val.astype(BF16)
            else:
                yacc[4 * r + n] = val

    def product(s, g, ab):
        prods, span = _plan(s)
        return _mm(lhs[prods.index(ab), 0:8 * (span[ab][1] - span[ab][0]) + 8], weight(g, ab))

    def ready_products(s):
        return [ab for ab in _plan(s)[0] if _mem_key(*ab, s) == (LEAD[(s - 1) % 4],)]

    def early_jobs(s):
        span = _plan(s)[1]
        longest = lambda ab: span[ab][0] - span[ab][1]
        jobs = [(g, ab) for g in EARLY_GROUPS for ab in sorted(ready_products(s), key=longest)[:2]]
        jobs = [job for i in range(0, len(jobs), 4) for job in sorted(jobs[i:i + 4], key=lambda j: longest(j[1]))]
        return {job: i for i, job in enumerate(jobs)}

    def go_ahead(s):
        for (g, ab), i in early_jobs(s).items():
            val = product(s, g, ab)
            v["ahead"][i, 0:val.shape[0]] = val

    def step(p, s):
        outer, inner = PHASE[s >> 1], PHASE[s & 1]
        prods, span = _plan(s)
        size = lambda ab: span[ab][1] - span[ab][0]
        prev, nxt = (s - 1) % 4, (s + 1) % 4
        mem_keys = sorted({_mem_key(*ab, s) for ab in prods})
        early = early_jobs(s)

        def project(g):
            res, mid = {}, {}
            for a in outer:
                for b in inner:
                    res[a, b] = (v["ahead"][early[g, (a, b)], 0:8 * size((a, b)) + 8] if (g, (a, b)) in early
                                 else product(s, g, (a, b)))
                mid[a] = _inner_blocks({(a, b): (*span[a, b], res[a, b][:-8]) for b in inner}, a)
                if a == outer[0]:
                    for j, (rn, (lo, hi, val)) in enumerate(mid[a].items()):
                        where = (4 * (g % 2) + j, slice(0, 8 * (hi - lo)))
                        v["parked"][where] = val
                        mid[a][rn] = (lo, hi, v["parked"][where])
                for r, n, terms in _outer_blocks(mid):
                    if a == [x for x in outer if (r >> 1, n >> 1) in STRASSEN[x][2]][-1]:
                        steps = _steps_touching(r, n)
                        if s != steps[0]:
                            terms = [(1, (0, 4, part[g, 4 * r + n]))] + terms
                        (fin if s == steps[-1] else part)[g, 4 * r + n] = _lin_rows(terms)[2]
            for n, val in enumerate(_mem_blocks({ab: val[-8:] for ab, val in res.items()}, s, range(4))):
                v["qkv_mem"][g, n] = val

        def rows(g, n):
            return [fin[g, 4 * nxt + n], v["qkv_mem"][g, n]]

        def scores(t):
            for n in range(4):
                q = jnp.concatenate(rows(t, n), 0)
                k = jnp.concatenate(rows(8 + t, n) + [pad], 0).astype(BF16)
                sc = jnp.where(keep, _mm_nt(q, k) * scale, fill)
                e = jnp.exp2(sc - jnp.max(sc, axis=1, keepdims=True))
                v["probs"][t, n] = e * pltpu.reciprocal(jnp.sum(e, axis=1, keepdims=True), approx=True)

        def values(t):
            if s == 0:
                o_old[t, 0:12] = o_new[t]
            om = []
            for n in range(4):
                o = _mm(v["probs"][t, n], jnp.concatenate(rows(16 + t, n) + [pad], 0).astype(BF16))
                (o_new if s else o_old)[t, 4 * prev + n] = o[:SEG]
                om.append(o[SEG:])
            for i, key in enumerate(mem_keys):
                v["o_mem"][t, i] = _lin([(1, om[c]) for c in key])

        def out_proj(half, ab):
            lo, hi = span[ab]
            rs = []
            for t in range(4 * half, 4 * half + 4):
                tok = _left_factors(lambda r, c: o_old[t, 4 * r + c, 8 * lo:8 * hi])(*ab)
                rs.append(_mm(jnp.concatenate([tok, v["o_mem"][t, mem_keys.index(_mem_key(*ab, s))]], 0),
                              weight(24 + t, ab)))
            total = (rs[0] + rs[1]) + (rs[2] + rs[3])
            where = (prods.index(ab), slice(0, 8 * size(ab) + 8))
            acc[where] = acc[where] + total if half else total

        def alternate(first):
            queue = {n: sorted((ab for ab in prods if size(ab) == n), key=lambda ab: ab not in first)
                     for n in (1, 2, 4)}
            return [queue[n].pop(0) for n in ROW_PATTERN]

        first_half = alternate(())
        for job in STEP_ORDER.split():
            kind, t = job[0], int(job[1:])
            if kind in "qkv":
                project(8 * "qkv".index(kind) + t)
            elif kind == "s":
                scores(t)
            elif kind == "p":
                values(t)
            elif kind == "x":
                xb[SEQ:SEQ + 8, 0:128] = acc[0, 0:8].astype(BF16)
                stage_tokens(p + (s == 3), nxt)
            else:
                for _ in range(t):
                    out_proj(0, first_half.pop(0))
        for i, ab in enumerate(alternate(lead_products(s))):
            out_proj(1, ab)
            if i == 13:
                stage_mem(nxt, new_mem(s, [LEAD[s]]), ready_products(nxt))
        go_ahead(nxt)
        stage_mem(nxt, new_mem(s, range(4)), [ab for ab in _plan(nxt)[0] if ab not in ready_products(nxt)])
        emit_tokens(p, s)

    wait(cp_x1)
    m0 = v["mem0"][...].astype(F32)
    stage_tokens(0, 0)
    stage_mem(0, [m0[:, _lanes(n)] for n in range(4)], _plan(0)[0])
    go_ahead(0)
    last = NSEG // 4 - 1

    @pl.loop(0, last + 1)
    def _(p):
        for s in range(4):
            step(p, s)
        pl.when(p == 0)(cp_x2.wait)
        pl.when(p > 0)(lambda: cp_yb(jnp.maximum(p - 1, 0)).start())

    tok = {}
    for ab in _products_without(3):
        rs = [_mm(_left_factors(lambda r, c: o_new[t, 4 * r + c], absent=3)(*ab), weight(24 + t, ab))
              for t in range(8)]
        tok[ab] = (0, 4, ((rs[0] + rs[1]) + (rs[2] + rs[3])) + ((rs[4] + rs[5]) + (rs[6] + rs[7])))
    for r, n, terms in _outer_blocks({a: _inner_blocks(tok, a) for a in range(7)}):
        if r < 3:
            yb[out_rows(last + 1, r), _lanes(n)] = _lin_rows(terms)[2].astype(BF16)
    cp_yb(last).start()
    wait(cp_ya)
    for p in range(last + 1):
        cp_yb(p).wait()


SCRATCH = {
    "xa": ((4, SEQ // 2, 128), U32),
    "feat": ((6, 64, 128), U32),
    "phase": (PHASES.shape, F32),
    "gmat": ((80, 64, 128), U32),
    "wr": ((16, 128, 128), U32),
    "wi": ((16, 128, 128), U32),
    "wnyq": ((2, 1, SEQ), BF16),
    "z_re": ((16, 264, 128), F32),
    "z_im": ((16, 264, 128), F32),
    "tmp": ((64, 128, 128), F32),
    "ya": ((4, SEQ // 2, 128), U32),
    "xb": ((SEQ + 16, DM), BF16),
    "mem0": ((NMEM, DM), BF16),
    "wsrc": ((24, DM // 4, 8, 128), U32),
    "wosrc": ((4, HEADS * DH // 2, 128), U32),
    "wc": ((32 * NPROD, 64, 128), U32),
    "lhs": ((16, LEN, 128), F32),
    "lhs0": ((NPROD, SEG, 128), F32),
    "part": ((24, 16, SEG, 128), F32),
    "fin": ((24, 16, SEG, 128), F32),
    "o_new": ((8, 12, SEG, 128), F32),
    "o_old": ((8, 16, SEG, 128), F32),
    "yacc": ((16, SEG, 128), F32),
    "yb": ((SEQ + 3 * SEG, DM), BF16),
    "qkv_mem": ((24, 4, 8, 128), F32),
    "probs": ((8, 4, LEN, 48), F32),
    "o_mem": ((8, 9, 8, 128), F32),
    "acc": ((16, LEN, 128), F32),
    "ahead": ((16, LEN, 128), F32),
    "parked": ((8, SEG, 128), F32),
    "spare": ((2, 8, 128), F32),
    "zero": None,
    "sems": None,
}


def _run(A_x, A_w_r, A_w_i, B_x, B_mem0, B_Wq, B_Wk, B_Wv, B_Wo):
    scratch = [pltpu.VMEM(*spec) for spec in SCRATCH.values() if spec]
    out = pl.pallas_call(
        _kernel,
        out_shape=jax.ShapeDtypeStruct((SEQ, 2 * DM), BF16),
        in_specs=[pl.BlockSpec(memory_space=pltpu.HBM)] * 10,
        out_specs=pl.BlockSpec(memory_space=pltpu.HBM),
        scratch_shapes=scratch + [pltpu.SMEM((1,), jnp.int32), pltpu.SemaphoreType.DMA((28,))],
        compiler_params=pltpu.CompilerParams(vmem_limit_bytes=120 * 2 ** 20),
    )(A_x.reshape(SEQ, DM), A_w_r.T, A_w_i.T, B_x.reshape(SEQ, DM), B_mem0.reshape(NMEM, DM),
      *(w.reshape(DM // 4, 4, HEADS, DH) for w in (B_Wq, B_Wk, B_Wv)),
      B_Wo.reshape(HEADS * DH, DM), PHASES)
    return out.reshape(1, SEQ, 2 * DM)


@jax.jit
def pallas_concat_heads__spectral_gfnet__memory_aug_recurrent_mem_tr__prompt_kernel(
    A_x: jax.Array,
    A_w_r: jax.Array,
    A_w_i: jax.Array,
    B_x: jax.Array,
    B_mem0: jax.Array,
    B_Wq: jax.Array,
    B_Wk: jax.Array,
    B_Wv: jax.Array,
    B_Wo: jax.Array,
    B_seg_len: jax.Array,
):
    del B_seg_len
    return _run(A_x, A_w_r, A_w_i, B_x, B_mem0, B_Wq, B_Wk, B_Wv, B_Wo)
```

```python
import itertools

import jax
import jax.numpy as jnp
import numpy as np
from jax import lax
from jax.experimental import pallas as pl
from jax.experimental.pallas import tpu as pltpu

F32, BF16, U32 = jnp.float32, jnp.bfloat16, jnp.uint32
SEQ, DM, HEADS, DH, NMEM, SEG = 2048, 512, 32, 128, 8, 32
NSEG = SEQ // SEG
LEN = NMEM + SEG
LOG2E = 1.4426950408889634

STRASSEN = (
    ({(0, 0): 1, (1, 1): 1}, {(0, 0): 1, (1, 1): 1}, {(0, 0): 1, (1, 1): 1}),
    ({(1, 0): 1, (1, 1): 1}, {(0, 0): 1}, {(1, 0): 1, (1, 1): -1}),
    ({(0, 0): 1}, {(0, 1): 1, (1, 1): -1}, {(0, 1): 1, (1, 1): 1}),
    ({(1, 1): 1}, {(1, 0): 1, (0, 0): -1}, {(0, 0): 1, (1, 0): 1}),
    ({(0, 0): 1, (0, 1): 1}, {(1, 1): 1}, {(0, 0): -1, (0, 1): 1}),
    ({(1, 0): 1, (0, 0): -1}, {(0, 0): 1, (0, 1): 1}, {(1, 1): 1}),
    ({(0, 1): 1, (1, 1): -1}, {(1, 0): 1, (1, 1): 1}, {(0, 0): 1}),
)
PHASE = ((4, 2, 6, 0), (1, 3, 5, 0))
PRODS = tuple(itertools.product(range(7), range(7)))
NPROD = len(PRODS)
LEAD = (3, 2, 1, 0)

STEP_ORDER = ("k0 q0 k1 q1 s0 v0 k2 s1 q2 p0 v1 k3 s2 p1 q3 v2 k4 s3 p2 q4 v3 k5 s4 p3 q5 v4 k6 s5 p4 "
              "q6 v5 k7 s6 p5 q7 v6 w4 s7 p6 v7 w4 x0 w4 p7 w4")
ROW_PATTERN = (4, 2, 4, 2, 4, 2, 4, 4, 1, 4, 2, 4, 2, 4, 2, 4)
EARLY_GROUPS = (8, 0, 9, 1, 16, 10, 2, 17)
BEAT_ORDER = {
    (0, 1, 3): "3012", (0, 2, 3): "0312", (0, 7, 0): "1203", (0, 8, 3): "0312", (0, 9, 2): "1023",
    (0, 10, 0): "0213", (0, 12, 1): "2103", (0, 14, 3): "0132", (0, 16, 1): "1023", (0, 19, 2): "2013",
    (0, 21, 1): "1023", (1, 0, 3): "0213", (1, 9, 3): "0132", (1, 10, 3): "0312", (1, 16, 0): "0213",
    (1, 17, 3): "0132", (1, 23, 3): "0312", (2, 2, 3): "0312", (2, 5, 3): "0132", (2, 6, 3): "0312",
    (2, 9, 2): "2103", (2, 10, 0): "1023", (2, 10, 3): "0312", (2, 11, 2): "1023", (2, 14, 2): "2013",
    (2, 18, 3): "3012", (2, 20, 2): "2013", (3, 2, 1): "2013", (3, 3, 3): "0213", (3, 7, 2): "0213",
    (3, 7, 3): "0132", (3, 10, 2): "2103", (3, 11, 3): "0213", (3, 13, 3): "0213", (3, 15, 3): "0312",
    (3, 16, 3): "0132",
}


def _rows_in_step(a, b, s):
    steps = [2 * p + q for p in range(2) for q in range(2) if a in PHASE[p] and b in PHASE[q]]
    k = steps.index(s)
    return k * 4 // len(steps), (k + 1) * 4 // len(steps)


def _plan(s):
    prods = [(a, b) for a in PHASE[s >> 1] for b in PHASE[s & 1]]
    return prods, {ab: _rows_in_step(*ab, s) for ab in prods}


def _steps_touching(r, n):
    return [s for s in range(4)
            if any((r >> 1, n >> 1) in STRASSEN[a][2] and (r & 1, n & 1) in STRASSEN[b][2] for a, b in _plan(s)[0])]


def _products_without(r):
    return [(a, b) for a, b in PRODS
            if all(any(2 * r1 + r2 != r for r1, _ in STRASSEN[a][k] for r2, _ in STRASSEN[b][k]) for k in (0, 2))]


def _mem_key(a, b, s):
    return tuple(sorted(2 * c1 + c2 for r1, c1 in STRASSEN[a][0] if r1 == s >> 1
                        for r2, c2 in STRASSEN[b][0] if r2 == s & 1))


def _lin(terms):
    terms = sorted(terms, key=lambda t: -t[0])
    c, x = terms[0]
    acc = x if c > 0 else -x
    for c, x in terms[1:]:
        acc = acc + x if c > 0 else acc - x
    return acc


def _lin_rows(terms):
    cuts = sorted({v for _, (lo, hi, _x) in terms for v in (lo, hi)})
    parts = [_lin([(c, x if (l, h) == (lo, hi) else x[8 * (lo - l):8 * (hi - l)])
                   for c, (l, h, x) in terms if l <= lo and hi <= h])
             for lo, hi in zip(cuts[:-1], cuts[1:])]
    return cuts[0], cuts[-1], parts[0] if len(parts) == 1 else jnp.concatenate(parts, 0)


def _inner_blocks(tok, a):
    out = {}
    for rn in itertools.product(range(2), range(2)):
        terms = [(STRASSEN[b][2][rn], tok[a, b]) for b in range(7) if rn in STRASSEN[b][2] and (a, b) in tok]
        if terms:
            out[rn] = _lin_rows(terms)
    return out


def _outer_blocks(mid):
    for r1, n1, r2, n2 in itertools.product(range(2), repeat=4):
        terms = [(STRASSEN[a][2][r1, n1], mid[a][r2, n2]) for a in mid
                 if (r1, n1) in STRASSEN[a][2] and (r2, n2) in mid[a]]
        if terms:
            yield 2 * r1 + r2, 2 * n1 + n2, terms


def _mem_blocks(res, s, ns):
    p, q, mid = s >> 1, s & 1, {}

    def inner(a, n2):
        if (a, n2) not in mid:
            mid[a, n2] = _lin([(STRASSEN[b][2][q, n2], res[a, b]) for b in PHASE[q] if (q, n2) in STRASSEN[b][2]])
        return mid[a, n2]
    return [_lin([(STRASSEN[a][2][p, n >> 1], inner(a, n & 1)) for a in PHASE[p] if (p, n >> 1) in STRASSEN[a][2]])
            for n in ns]


def _left_factors(get, absent=None):
    cache = {}

    def factor(a, b):
        terms = []
        for (r2, c2), cb in STRASSEN[b][0].items():
            if (a, r2, c2) not in cache:
                part = [(ca, get(2 * r1 + r2, 2 * c1 + c2)) for (r1, c1), ca in STRASSEN[a][0].items()
                        if 2 * r1 + r2 != absent]
                cache[a, r2, c2] = _lin(part) if part else None
            if cache[a, r2, c2] is not None:
                terms.append((cb, cache[a, r2, c2]))
        return _lin(terms)
    return factor


def _mm(a, b):
    return jnp.dot(a, b, preferred_element_type=F32)


def _mm_nt(a, b):
    return lax.dot_general(a, b, (((1,), (1,)), ((), ())), preferred_element_type=F32)


def _lo(u):
    return lax.bitcast_convert_type(u << 16, F32)


def _hi(u):
    return lax.bitcast_convert_type(u & np.uint32(0xFFFF0000), F32)


def _pack(both):
    return pltpu.bitcast(both.astype(BF16).reshape(2 * both.shape[0], 128), U32)


def _lanes(c):
    return slice(128 * c, 128 * (c + 1))


def _twiddle(z, k, sign):
    k = (k * sign) % 16
    re, im = z
    if k == 0:
        return re, im
    if k % 4 == 0:
        return (-im, re) if k == 4 else (-re, -im) if k == 8 else (im, -re)
    c, s = float(np.cos(np.pi * k / 8)), float(np.sin(np.pi * k / 8))
    if k % 4 == 2:
        return ((re - im) * c, (re + im) * c) if c * s > 0 else ((re + im) * c, (im - re) * c)
    return re * c - im * s, re * s + im * c


def _dft4(z, sign):
    (ar, ai), (br, bi), (cr, ci), (dr, di) = z
    pr, pi, mr, mi = ar + cr, ai + ci, ar - cr, ai - ci
    qr, qi, nr, ni = br + dr, bi + di, br - dr, bi - di
    up, dn = (mr - ni, mi + nr), (mr + ni, mi - nr)
    return [(pr + qr, pi + qi), up if sign > 0 else dn, (pr - qr, pi - qi), dn if sign > 0 else up]


def _dft16(z, sign):
    cols = [_dft4([z[n2 + 4 * n1] for n1 in range(4)], sign) for n2 in range(4)]
    out = [None] * 16
    for k1 in range(4):
        for k2, val in enumerate(_dft4([_twiddle(cols[n2][k1], n2 * k1, sign) for n2 in range(4)], sign)):
            out[k1 + 4 * k2] = val
    return out


def _phase_table():
    freq = np.concatenate([np.arange(0, 16, 2) / 128, np.arange(1, 16, 2) / 128, np.arange(8) / 8,
                           np.arange(16) / SEQ])
    angle = 2 * np.pi * freq[:, None] * np.arange(128)[None, :]
    return np.stack([np.cos(angle), -np.sin(angle)]).astype(np.float32)


PHASES = _phase_table()


def _dft_matrices(table, feat, gmat):
    def times(x, row):
        tr, ti = (jnp.concatenate([table[c, row:row + 1]] * 2, 1) for c in range(2))
        return x[0] * tr - x[1] * ti, x[0] * ti + x[1] * tr

    low = [jnp.concatenate([table[c, 0:8], table[c, 8:16]], 1) for c in range(2)]
    base = [jnp.concatenate(part, 0) for part in zip(*(times(low, 16 + i) for i in range(8)))]
    norm = 2.0 / (SEQ * DM)
    for a in range(16):
        gr, gi = times(base, 24 + a)
        for j, g in enumerate((gr, gi - gr, gr + gi, gr * norm, gi * norm)):
            gmat[5 * a + j] = _pack(g)
        cos, nsin = gr[:32], gi[:32]
        if a == 0:
            row, col = (lax.broadcasted_iota(jnp.int32, (32, 256), d) for d in range(2))
            nsin = jnp.where((row == 0) & (col < 128), (1 - 2 * (col & 1)).astype(F32), nsin)
        for j, halves in {0: {0: (cos, nsin)}, 8: {1: (cos, nsin)}, 4: {2: (cos, nsin), 4: (nsin, -cos)},
                          12: {3: (cos, nsin), 5: (-nsin, cos)}}.get(a, {}).items():
            feat[j] = _pack(jnp.concatenate(halves, 0))


def _spectral(v, wait_filter, split_code):
    z_re, z_im, tmp = v["z_re"], v["z_im"], v["tmp"]
    sublane = lax.broadcasted_iota(jnp.int32, (8, 128), 0)
    first, never = sublane == 0, sublane < v["zero"][0]
    dmat = lambda i: pltpu.bitcast(v["feat"][i], BF16)
    smat = lambda a, j: pltpu.bitcast(v["gmat"][5 * a + j], BF16)

    for j in range(8):
        words = [v["xa"][c, pl.ds(j, 128, stride=8), :] for c in range(4)]
        for half, unpack in enumerate((_lo, _hi)):
            a = 2 * j + half
            x0, x1, x2, x3 = [unpack(w) for w in words]
            p, q = x0 + x2, x1 + x3
            u, w = (x0 - x2).astype(BF16), (x1 - x3).astype(BF16)
            rs = (_mm_nt(dmat(0), (p + q).astype(BF16)), _mm_nt(dmat(2), u) + _mm_nt(dmat(4), w),
                  _mm_nt(dmat(1), (p - q).astype(BF16)), _mm_nt(dmat(3), u) + _mm_nt(dmat(5), w))
            for r, val in enumerate(rs):
                z_re[a, 8 + 64 * r:72 + 64 * r] = val[:64]
                z_im[a, 8 + 64 * r:72 + 64 * r] = val[64:] if r else jnp.concatenate(
                    [jnp.where(first, 0.0, val[64:72]), val[72:]], 0)
            z_re[a, 0:8] = jnp.where(first, rs[0][64:72], 0.0)

    def forward(r):
        body = slice(8 + 64 * r, 72 + 64 * r)
        rows = body if r else slice(0, 72)
        add = lambda x, y: x + y if r else jnp.concatenate([x[:8], x[8:] + y], 0)
        for a in range(16):
            ure, uim = z_re[a, rows], z_im[a, body]
            both = _mm(add(ure, uim), smat(a, 0))
            z_im[a, rows] = both + _mm(ure, smat(a, 1))
            z_re[a, rows] = val = add(both, -_mm(uim, smat(a, 2)))
            yield val[56:64]

    def inverse(r):
        for a in range(16):
            zr, zi = z_re[a, 8 + 64 * r:72 + 64 * r], z_im[a, 8 + 64 * r:72 + 64 * r]
            bot_r, bot_i = zi, -zr
            if r == 0:
                head = lambda new, old: jnp.concatenate([jnp.where(first, 0.5 * new, old[:8]), old[8:]], 0)
                bot_r, bot_i = head(z_re[a, 0:8], bot_r), head(z_im[a, 0:8], bot_i)
                zr, zi = head(zr[:8], zr), head(zi[:8], zi)
            tmp[4 * a + r] = val = (_mm_nt(smat(a, 3), jnp.concatenate([zr, bot_r], 0).astype(BF16))
                                    + _mm_nt(smat(a, 4), jnp.concatenate([zi, bot_i], 0).astype(BF16)))
            yield val[56:64]

    def mix(row, weight, pace=None):
        z = [(z_re[a, row:row + 8], z_im[a, row:row + 8]) for a in range(16)]
        if pace:
            z[0] = (jnp.where(never, pace[0], z[0][0]), z[0][1])
        y = []
        for k, (xr, xi) in enumerate(_dft16(z, -1)):
            cr, ci = weight(k)
            y.append((xr * cr - xi * ci, xr * ci + xi * cr))
        if pace:
            y[0] = (jnp.where(never, pace[1], y[0][0]), y[0][1])
        for a, (yr, yi) in enumerate(_dft16(y, 1)):
            z_re[a, row:row + 8] = yr
            z_im[a, row:row + 8] = yi

    def apply_filter(r, matmuls):
        if r == 0:
            mix(0, lambda k: tuple(jnp.where(first, v["wnyq"][c, :, _lanes(k)].astype(F32), 0.0) for c in range(2)))
        unpack = (_lo, _hi)[r & 1]
        for blk in range(8):
            src = pl.ds(16 * blk + (r >> 1), 8, stride=2)
            mix(8 + 64 * r + 8 * blk, lambda k: (unpack(v["wr"][k, src, :]), unpack(v["wi"][k, src, :])),
                [next(matmuls), next(matmuls)])

    list(forward(0))
    wait_filter()
    apply_filter(0, forward(1))
    apply_filter(1, forward(2))
    split_code()
    apply_filter(2, forward(3))
    apply_filter(3, inverse(0))
    for r in range(1, 4):
        list(inverse(r))

    for j in range(8):
        u = [[tmp[4 * (2 * j + half) + r] for r in range(4)] for half in range(2)]
        ea = [_mm(x[0], dmat(0)) for x in u]
        eb = [_mm(x[2], dmat(1)) for x in u]
        for c in range(2):
            even = [p - q if c else p + q for p, q in zip(ea, eb)]
            odd = [_mm(x[1], dmat(2 + 2 * c)) + _mm(x[3], dmat(3 + 2 * c)) for x in u]
            v["ya"][c, pl.ds(j, 128, stride=8), :] = _pack(jnp.concatenate([even[0] + odd[0], even[1] + odd[1]], 1))
            v["ya"][c + 2, pl.ds(j, 128, stride=8), :] = _pack(jnp.concatenate([even[0] - odd[0], even[1] - odd[1]], 1))


def _combine_weights(load, wc, base, matmuls, never):
    issued = [None]
    for i in range(8):
        issued.append(next(matmuls, None))
        pace, blk = issued.pop(0), {}
        for a in (0, 1, 4, 2, 5, 3, 6):
            for c1, n1 in STRASSEN[a][1]:
                if (2 * c1, 2 * n1) not in blk:
                    blk.update(load(i, c1, n1))
                    if pace is not None and (c1, n1) == (1, 0):
                        x = blk[2, 0]
                        blk[2, 0] = jnp.concatenate([jnp.where(never, pace, x[:, :128]), x[:, 128:]], 1)
            mid = {(c2, n2): _lin([(k, blk[2 * c1 + c2, 2 * n1 + n2]) for (c1, n1), k in STRASSEN[a][1].items()])
                   for c2 in range(2) for n2 in range(2)}
            for b in range(7):
                wc[base + 7 * a + b, 8 * i:8 * i + 8, :] = _pack(
                    _lin([(k, mid[cn]) for cn, k in STRASSEN[b][1].items()]))


def _kernel(ax_hbm, wr_hbm, wi_hbm, x_hbm, mem_hbm, wq_hbm, wk_hbm, wv_hbm, wo_hbm, phase_hbm,
            out_hbm, *scratch):
    v = dict(zip(SCRATCH, scratch))
    xb, yb, wc, sems = v["xb"], v["yb"], v["wc"], v["sems"]
    lhs, part, fin, o_new, o_old, acc, yacc = (v[k] for k in ("lhs", "part", "fin", "o_new", "o_old", "acc", "yacc"))
    copy = pltpu.make_async_copy

    cp_phase = copy(phase_hbm, v["phase"], sems.at[0])
    cp_x0 = copy(x_hbm.at[0:3 * SEG], xb.at[0:3 * SEG], sems.at[1])
    cp_ax = [copy(ax_hbm.bitcast(U32).at[:, _lanes(c)], v["xa"].at[c], sems.at[2]) for c in range(4)]
    cp_filter = [copy(src.at[0:256].bitcast(U32).at[:, _lanes(k)], dst.at[k], sems.at[3])
                 for src, dst in ((wr_hbm, v["wr"]), (wi_hbm, v["wi"])) for k in range(16)]
    cp_filter += [copy(src.at[256:257, :], v["wnyq"].at[c], sems.at[3]) for c, src in enumerate((wr_hbm, wi_hbm))]
    cp_qkv = [[[copy(src.bitcast(U32).at[:, q, 4 * h:4 * h + 4, :],
                     v["wsrc"].at[8 * w + 2 * h + q % 2, :, 4 * (q // 2):4 * (q // 2) + 4, :], sems.at[4 + 4 * w + h])
                for q in range(4)] for h in range(4)] for w, src in enumerate((wq_hbm, wk_hbm, wv_hbm))]
    cp_wo = [[copy(wo_hbm.bitcast(U32).at[256 * t:256 * t + 256, _lanes(c)],
                   v["wosrc"].at[c, 256 * t:256 * t + 256], sems.at[16 + t]) for c in range(4)] for t in range(8)]
    cp_x1 = [copy(x_hbm.at[3 * SEG:7 * SEG], xb.at[3 * SEG:7 * SEG], sems.at[24]),
             copy(mem_hbm, v["mem0"], sems.at[24])]
    cp_x2 = copy(x_hbm.at[7 * SEG:11 * SEG], xb.at[7 * SEG:11 * SEG], sems.at[25])
    cp_x3 = copy(x_hbm.at[11 * SEG:SEQ], xb.at[11 * SEG:SEQ], sems.at[28])
    cp_ya = [copy(v["ya"].at[c], out_hbm.bitcast(U32).at[:, _lanes(c)], sems.at[26]) for c in range(4)]

    def cp_yb(p):
        return copy(yb.at[pl.ds(pl.multiple_of(p * 128 + 3 * SEG, SEG), 128)],
                    out_hbm.at[pl.ds(pl.multiple_of(p * 128, 128), 128), DM:2 * DM], sems.at[27])

    def start(copies):
        for c in copies:
            c.start()

    def wait(copies):
        for c in copies:
            c.wait()

    start([cp_phase, cp_x0] + cp_ax + cp_filter + sum(cp_qkv[0], []))
    v["zero"][0] = 0

    @pl.loop(0, 2)
    def _(i):
        zero = jnp.zeros((8, 128), F32)
        for k in ("lhs", "yacc", "acc", "ahead", "parked", "tmp", "z_re", "z_im"):
            v[k][i, 0:8] = zero
        for k in ("part", "o_old", "qkv_mem", "o_mem"):
            v[k][i, 0, 0:8] = zero
        v["probs"][i, 0, 0:8] = zero[:, :48]
        for k in ("gmat", "feat"):
            v[k][i, 0:8] = lax.bitcast_convert_type(zero, U32)

    weight = lambda g, ab: pltpu.bitcast(wc[g * NPROD + 7 * ab[0] + ab[1]], BF16)

    def x_blocks(seg_of):
        cache = {}

        def get(r, c):
            if r not in cache:
                cache[r] = xb[pl.ds(pl.multiple_of(seg_of(r) * SEG, SEG), SEG), :].astype(F32)
            return cache[r][:, _lanes(c)]
        return get

    o_new[...] = jnp.zeros(o_new.shape, F32)
    cp_x0.wait()
    first_prods = _products_without(0)
    factor = _left_factors(x_blocks(lambda r: r - 1), absent=0)
    for a, b in first_prods:
        v["lhs0"][7 * a + b] = factor(a, b)
    cp_phase.wait()
    _dft_matrices(v["phase"], v["feat"], v["gmat"])
    wait(cp_ax)

    def wait_filter():
        wait(cp_filter)
        start(sum(cp_qkv[1] + cp_qkv[2], []))

    def split_code():
        @pl.loop(0, 2)
        def _(i):
            v["spare"][i] = jnp.zeros((8, 128), F32)

    _spectral(v, wait_filter, split_code)

    wrows = v["wsrc"].reshape(24, DM * 2, 128)

    def load_qkv(w, t):
        def load(i, c1, n1):
            blk = {}
            for kt in (2 * c1, 2 * c1 + 1):
                rows = pl.ds((64 * kt + 8 * i) * 4 + 2 * (t % 2) + n1, 8, stride=4)
                u = jnp.concatenate([wrows[8 * w + 2 * (t // 2) + par, rows, :] for par in range(2)], 1)
                blk[kt, 2 * n1], blk[kt, 2 * n1 + 1] = _lo(u), _hi(u)
            return blk
        return load

    def load_out(t):
        def load(i, c1, n1):
            blk = {}
            for hd in (2 * c1, 2 * c1 + 1):
                for n in (2 * n1, 2 * n1 + 1):
                    u = v["wosrc"][n, pl.ds((4 * t + hd) * 64 + 8 * i, 8), :]
                    blk[hd, n] = jnp.concatenate([_lo(u), _hi(u)], 1)
            return blk
        return load

    def first_tokens(g):
        seen = set()
        for a in range(7):
            tok = {(a, b): (0, 4, _mm(v["lhs0"][7 * a + b], weight(g, (a, b))))
                   for b in (4, 2, 6, 0, 3, 1, 5) if (a, b) in first_prods}
            for r, n, terms in _outer_blocks({a: _inner_blocks(tok, a)}):
                if r:
                    if (r, n) in seen:
                        terms = [(1, (0, 4, fin[g, 4 * r + n]))] + terms
                    seen.add((r, n))
                    fin[g, 4 * r + n] = val = _lin_rows(terms)[2]
            yield val[24:32]

    arrived = {0: cp_qkv[0], 8: cp_qkv[1], 16: cp_qkv[2][:2], 20: cp_qkv[2][2:],
               24: cp_wo[:2], 26: cp_wo[2:4], 28: cp_wo[4:6], 30: cp_wo[6:7], 31: cp_wo[7:]}
    never = lax.broadcasted_iota(jnp.int32, (8, 128), 0) < v["zero"][0]
    for g in range(32):
        if g == 16:
            start(sum(cp_wo, []) + cp_x1 + [cp_x2])
        if g == 20:
            split_code()
        wait(sum(arrived.get(g, []), []))
        _combine_weights(load_qkv(g // 8, g % 8) if g < 24 else load_out(g % 8), wc, g * NPROD,
                         first_tokens(g - 8) if 8 <= g < 31 else iter(()), never)
        if g == 27:
            list(first_tokens(23))
    start([cp_x3] + cp_ya)

    row = lax.broadcasted_iota(jnp.int32, (LEN, 48), 0)
    col = lax.broadcasted_iota(jnp.int32, (LEN, 48), 1)
    keep = ((row >= SEG) | (col >= SEG) | (row >= col)) & (col < LEN)
    fill = jnp.where(col < LEN, -1e9 * LOG2E, -jnp.inf).astype(F32)
    scale = DH ** -0.5 * LOG2E
    pad = jnp.zeros((8, 128), F32)

    def out_rows(p, r):
        return pl.ds(pl.multiple_of(p * 128 + r * SEG, SEG), SEG)

    def stage_tokens(p, s):
        prods, span = _plan(s)
        factor = _left_factors(x_blocks(lambda r: jnp.minimum(4 * p + 3 + r, NSEG - 1)))
        for i, ab in enumerate(prods):
            lo, hi = span[ab]
            lhs[i, 0:8 * (hi - lo)] = factor(*ab)[8 * lo:8 * hi]

    def stage_mem(s, mem, which):
        prods, span = _plan(s)
        for i, ab in enumerate(prods):
            if ab in which:
                n = 8 * (span[ab][1] - span[ab][0])
                lhs[i, n:n + 8] = _lin([(1, mem[c]) for c in _mem_key(*ab, s)])

    def lead_products(s):
        return [ab for ab in _plan(s)[0] if (s >> 1, LEAD[s] >> 1) in STRASSEN[ab[0]][2]
                and (s & 1, LEAD[s] & 1) in STRASSEN[ab[1]][2]]

    def new_mem(s, ns):
        prods, span = _plan(s)
        res = {ab: acc[i, 8 * (span[ab][1] - span[ab][0]):8 * (span[ab][1] - span[ab][0]) + 8]
               for i, ab in enumerate(prods) if len(ns) > 1 or ab in lead_products(s)}
        return dict(zip(ns, _mem_blocks(res, s, ns)))

    def emit_tokens(p, s):
        prods, span = _plan(s)
        tok = {ab: (*span[ab], acc[i, 0:8 * (span[ab][1] - span[ab][0])]) for i, ab in enumerate(prods)}
        for r, n, terms in _outer_blocks({a: _inner_blocks(tok, a) for a in PHASE[s >> 1]}):
            steps = _steps_touching(r, n)
            if s != steps[0]:
                terms = [(1, (0, 4, yacc[4 * r + n]))] + terms
            val = _lin_rows(terms)[2]
            if s == steps[-1]:
                yb[out_rows(p, r), _lanes(n)] = val.astype(BF16)
            else:
                yacc[4 * r + n] = val

    def product(s, g, ab):
        prods, span = _plan(s)
        return _mm(lhs[prods.index(ab), 0:8 * (span[ab][1] - span[ab][0]) + 8], weight(g, ab))

    def ready_products(s):
        return [ab for ab in _plan(s)[0] if _mem_key(*ab, s) == (LEAD[(s - 1) % 4],)]

    def early_jobs(s):
        span = _plan(s)[1]
        longest = lambda ab: span[ab][0] - span[ab][1]
        jobs = [(g, ab) for g in EARLY_GROUPS for ab in sorted(ready_products(s), key=longest)[:2]]
        jobs = [job for i in range(0, len(jobs), 4) for job in sorted(jobs[i:i + 4], key=lambda j: longest(j[1]))]
        return {job: i for i, job in enumerate(jobs)}

    def go_ahead(s):
        for (g, ab), i in early_jobs(s).items():
            val = product(s, g, ab)
            v["ahead"][i, 0:val.shape[0]] = val

    def step(p, s):
        outer, inner = PHASE[s >> 1], PHASE[s & 1]
        prods, span = _plan(s)
        size = lambda ab: span[ab][1] - span[ab][0]
        prev, nxt = (s - 1) % 4, (s + 1) % 4
        mem_keys = sorted({_mem_key(*ab, s) for ab in prods})
        early = early_jobs(s)

        def project(g):
            res, mid = {}, {}
            for a in outer:
                for b in [inner[int(i)] for i in BEAT_ORDER.get((s, g, outer.index(a)), "0123")]:
                    res[a, b] = (v["ahead"][early[g, (a, b)], 0:8 * size((a, b)) + 8] if (g, (a, b)) in early
                                 else product(s, g, (a, b)))
                mid[a] = _inner_blocks({(a, b): (*span[a, b], res[a, b][:-8]) for b in inner}, a)
                if a == outer[0]:
                    for j, (rn, (lo, hi, val)) in enumerate(mid[a].items()):
                        where = (4 * (g % 2) + j, slice(0, 8 * (hi - lo)))
                        v["parked"][where] = val
                        mid[a][rn] = (lo, hi, v["parked"][where])
                for r, n, terms in _outer_blocks(mid):
                    if a == [x for x in outer if (r >> 1, n >> 1) in STRASSEN[x][2]][-1]:
                        steps = _steps_touching(r, n)
                        if s != steps[0]:
                            terms = [(1, (0, 4, part[g, 4 * r + n]))] + terms
                        (fin if s == steps[-1] else part)[g, 4 * r + n] = _lin_rows(terms)[2]
            for n, val in enumerate(_mem_blocks({ab: val[-8:] for ab, val in res.items()}, s, range(4))):
                v["qkv_mem"][g, n] = val

        def rows(g, n):
            return [fin[g, 4 * nxt + n], v["qkv_mem"][g, n]]

        def scores(t):
            for n in range(4):
                q = jnp.concatenate(rows(t, n), 0)
                k = jnp.concatenate(rows(8 + t, n) + [pad], 0).astype(BF16)
                sc = jnp.where(keep, _mm_nt(q, k) * scale, fill)
                e = jnp.exp2(sc - jnp.max(sc, axis=1, keepdims=True))
                v["probs"][t, n] = e * pltpu.reciprocal(jnp.sum(e, axis=1, keepdims=True), approx=True)

        def values(t):
            if s == 0:
                o_old[t, 0:12] = o_new[t]
            om = []
            for n in range(4):
                o = _mm(v["probs"][t, n], jnp.concatenate(rows(16 + t, n) + [pad], 0).astype(BF16))
                (o_new if s else o_old)[t, 4 * prev + n] = o[:SEG]
                om.append(o[SEG:])
            for i, key in enumerate(mem_keys):
                v["o_mem"][t, i] = _lin([(1, om[c]) for c in key])

        def out_proj(half, ab):
            lo, hi = span[ab]
            rs = []
            for t in range(4 * half, 4 * half + 4):
                tok = _left_factors(lambda r, c: o_old[t, 4 * r + c, 8 * lo:8 * hi])(*ab)
                rs.append(_mm(jnp.concatenate([tok, v["o_mem"][t, mem_keys.index(_mem_key(*ab, s))]], 0),
                              weight(24 + t, ab)))
            total = (rs[0] + rs[1]) + (rs[2] + rs[3])
            where = (prods.index(ab), slice(0, 8 * size(ab) + 8))
            acc[where] = acc[where] + total if half else total

        def alternate(first):
            queue = {n: sorted((ab for ab in prods if size(ab) == n), key=lambda ab: ab not in first)
                     for n in (1, 2, 4)}
            return [queue[n].pop(0) for n in ROW_PATTERN]

        first_half = alternate(())
        for job in STEP_ORDER.split():
            kind, t = job[0], int(job[1:])
            if kind in "qkv":
                project(8 * "qkv".index(kind) + t)
            elif kind == "s":
                scores(t)
            elif kind == "p":
                values(t)
            elif kind == "x":
                xb[SEQ:SEQ + 8, 0:128] = acc[0, 0:8].astype(BF16)
                stage_tokens(p + (s == 3), nxt)
            else:
                for _ in range(t):
                    out_proj(0, first_half.pop(0))
        for i, ab in enumerate(alternate(lead_products(s))):
            out_proj(1, ab)
            if i == 13:
                stage_mem(nxt, new_mem(s, [LEAD[s]]), ready_products(nxt))
        go_ahead(nxt)
        stage_mem(nxt, new_mem(s, range(4)), [ab for ab in _plan(nxt)[0] if ab not in ready_products(nxt)])
        emit_tokens(p, s)

    wait(cp_x1)
    m0 = v["mem0"][...].astype(F32)
    stage_tokens(0, 0)
    stage_mem(0, [m0[:, _lanes(n)] for n in range(4)], _plan(0)[0])
    go_ahead(0)
    cp_x2.wait()
    last = NSEG // 4 - 1

    @pl.loop(0, last + 1)
    def _(p):
        for s in range(4):
            step(p, s)
        pl.when(p > 0)(lambda: cp_yb(jnp.maximum(p - 1, 0)).start())
        pl.when(p == 0)(cp_x3.wait)

    tok = {}
    for ab in _products_without(3):
        rs = [_mm(_left_factors(lambda r, c: o_new[t, 4 * r + c], absent=3)(*ab), weight(24 + t, ab))
              for t in range(8)]
        tok[ab] = (0, 4, ((rs[0] + rs[1]) + (rs[2] + rs[3])) + ((rs[4] + rs[5]) + (rs[6] + rs[7])))
    for r, n, terms in _outer_blocks({a: _inner_blocks(tok, a) for a in range(7)}):
        if r < 3:
            yb[out_rows(last + 1, r), _lanes(n)] = _lin_rows(terms)[2].astype(BF16)
    cp_yb(last).start()
    wait(cp_ya)
    for p in range(last + 1):
        cp_yb(p).wait()


SCRATCH = {
    "xa": ((4, SEQ // 2, 128), U32),
    "feat": ((6, 64, 128), U32),
    "phase": (PHASES.shape, F32),
    "gmat": ((80, 64, 128), U32),
    "wr": ((16, 128, 128), U32),
    "wi": ((16, 128, 128), U32),
    "wnyq": ((2, 1, SEQ), BF16),
    "z_re": ((16, 264, 128), F32),
    "z_im": ((16, 264, 128), F32),
    "tmp": ((64, 128, 128), F32),
    "ya": ((4, SEQ // 2, 128), U32),
    "xb": ((SEQ + 16, DM), BF16),
    "mem0": ((NMEM, DM), BF16),
    "wsrc": ((24, DM // 4, 8, 128), U32),
    "wosrc": ((4, HEADS * DH // 2, 128), U32),
    "wc": ((32 * NPROD, 64, 128), U32),
    "lhs": ((16, LEN, 128), F32),
    "lhs0": ((NPROD, SEG, 128), F32),
    "part": ((24, 16, SEG, 128), F32),
    "fin": ((24, 16, SEG, 128), F32),
    "o_new": ((8, 12, SEG, 128), F32),
    "o_old": ((8, 16, SEG, 128), F32),
    "yacc": ((16, SEG, 128), F32),
    "yb": ((SEQ + 3 * SEG, DM), BF16),
    "qkv_mem": ((24, 4, 8, 128), F32),
    "probs": ((8, 4, LEN, 48), F32),
    "o_mem": ((8, 9, 8, 128), F32),
    "acc": ((16, LEN, 128), F32),
    "ahead": ((16, LEN, 128), F32),
    "parked": ((8, SEG, 128), F32),
    "spare": ((2, 8, 128), F32),
    "zero": None,
    "sems": None,
}


def _run(A_x, A_w_r, A_w_i, B_x, B_mem0, B_Wq, B_Wk, B_Wv, B_Wo):
    scratch = [pltpu.VMEM(*spec) for spec in SCRATCH.values() if spec]
    out = pl.pallas_call(
        _kernel,
        out_shape=jax.ShapeDtypeStruct((SEQ, 2 * DM), BF16),
        in_specs=[pl.BlockSpec(memory_space=pltpu.HBM)] * 10,
        out_specs=pl.BlockSpec(memory_space=pltpu.HBM),
        scratch_shapes=scratch + [pltpu.SMEM((1,), jnp.int32), pltpu.SemaphoreType.DMA((29,))],
        compiler_params=pltpu.CompilerParams(vmem_limit_bytes=120 * 2 ** 20),
    )(A_x.reshape(SEQ, DM), A_w_r.T, A_w_i.T, B_x.reshape(SEQ, DM), B_mem0.reshape(NMEM, DM),
      *(w.reshape(DM // 4, 4, HEADS, DH) for w in (B_Wq, B_Wk, B_Wv)),
      B_Wo.reshape(HEADS * DH, DM), PHASES)
    return out.reshape(1, SEQ, 2 * DM)


@jax.jit
def pallas_concat_heads__spectral_gfnet__memory_aug_recurrent_mem_tr__prompt_kernel(
    A_x: jax.Array,
    A_w_r: jax.Array,
    A_w_i: jax.Array,
    B_x: jax.Array,
    B_mem0: jax.Array,
    B_Wq: jax.Array,
    B_Wk: jax.Array,
    B_Wv: jax.Array,
    B_Wo: jax.Array,
    B_seg_len: jax.Array,
):
    del B_seg_len
    return _run(A_x, A_w_r, A_w_i, B_x, B_mem0, B_Wq, B_Wk, B_Wv, B_Wo)
```
